```python
import os as _os
_os.environ.setdefault("JAX_PLATFORMS", "cpu")
import jax
import jax.numpy as jnp

def _softmax(x, axis=-1):
    return jax.nn.softmax(x, axis=axis)
def _gelu(x):
    return jax.nn.gelu(x, approximate=True)
def _silu(x):
    return jax.nn.silu(x)
def _sigmoid(x):
    return jax.nn.sigmoid(x)
def _layernorm(x, axis=-1, eps=1e-5):
    m = jnp.mean(x, axis=axis, keepdims=True)
    v = jnp.var(x, axis=axis, keepdims=True)
    return (x - m) / jnp.sqrt(v + eps)
def _scatter_add(tgt, idx, src, axis=0):
    return tgt.at[idx].add(src)
def _segment_sum(src, seg, n):
    return jax.ops.segment_sum(src, seg, n)
class _Rng:
    def __init__(self, key):
        self._k = key
    def _next(self):
        self._k, sub = jax.random.split(self._k)
        return sub
    def normal(self, shape):
        return jax.random.normal(self._next(), shape, dtype=jnp.bfloat16)
    def randint(self, lo, hi, shape):
        return jax.random.randint(self._next(), shape, lo, hi, dtype=jnp.int32)
    def uniform(self, shape, lo=0.0, hi=1.0):
        return jax.random.uniform(self._next(), shape, jnp.bfloat16, lo, hi)
    def permutation(self, n):
        return jax.random.permutation(self._next(), n)


kernel_name = 'gated_mix__ssm_conv_h3__spectral_gfnet__prompt'

def setup_inputs():
    _rng = _Rng(jax.random.key(int.from_bytes(__import__("os").urandom(4), "little")))
    _w = (lambda a: (lambda t: t.astype(jnp.bfloat16) if jnp.issubdtype(t.dtype, jnp.floating) else t)(jnp.asarray(a)))
    def _A_setup():
        B, S, D = 1, 2048, 1024
        ks = 4
        return {
            "q": _w((lambda *s: _rng.normal(s) * 0.05)(B, S, D)),
            "k": _w((lambda *s: _rng.normal(s) * 0.1)(B, S, D)),
            "v": _w((lambda *s: _rng.normal(s) * 0.1)(B, S, D)),
            "shift_k": _w((lambda *s: _rng.normal(s) * 0.1)(D, ks) * 0.5),
            "ssm_k": _w((lambda *s: _rng.normal(s) * 0.1)(D, S) * (1.0 / S ** 0.5)),
            "ssm_D": _w((lambda *s: _rng.normal(s) * 0.1)(D)),
        }
    _A_in = _A_setup()

    def _B_setup():
        B, S, D = 1, 2048, 1024
        Df = D // 2 + 1
        return {
            "x": _w((lambda *s: _rng.normal(s) * 0.05)(B, S, D)),
            "w_r": _w((lambda *s: _rng.normal(s) * 0.05)(S, Df) * 0.02),
            "w_i": _w((lambda *s: _rng.normal(s) * 0.05)(S, Df) * 0.02),
        }
    _B_in = _B_setup()

    return {
        "A_q": _A_in["q"],
        "A_k": _A_in["k"],
        "A_v": _A_in["v"],
        "A_shift_k": _A_in["shift_k"],
        "A_ssm_k": _A_in["ssm_k"],
        "A_ssm_D": _A_in["ssm_D"],
        "B_x": _B_in["x"],
        "B_w_r": _B_in["w_r"],
        "B_w_i": _B_in["w_i"],
        "gate_w": _w((lambda *s: _rng.normal(s) * 0.05)(1024) * 16.0),
    }

def reference(A_q, A_k, A_v, A_shift_k, A_ssm_k, A_ssm_D, B_x, B_w_r, B_w_i, gate_w):
    def _A_ref(q, k, v, shift_k, ssm_k, ssm_D):
        B, S, D = q.shape
        ks = shift_k.shape[-1]
        k_pad = jnp.pad(k, ((0, 0), (ks - 1, 0), (0, 0)))
        k_shift = jnp.zeros_like(k)
        for t in range(ks):
            k_shift = k_shift + k_pad[:, t:t + S, :] * shift_k[:, ks - 1 - t][None, None, :]
        kv = k_shift * v
        L = 2 * S
        kv_pad = jnp.pad(kv, ((0, 0), (0, S), (0, 0)))
        kf_pad = jnp.pad(ssm_k, ((0, 0), (0, S)))
        kv_f = (lambda x, axes=(-2,-1): jnp.fft.rfft2(x.astype(jnp.float32), axes=axes))(kv_pad[:, None, :, :], axes=(1, 2))
        kf_f = (lambda x, axes=(-2,-1): jnp.fft.rfft2(x.astype(jnp.float32), axes=axes))(kf_pad[:, None, :], axes=(1, 2))
        kf_f = (lambda x, *d: x.transpose(*d))(kf_f, 1, 2, 0)
        y_f = kv_f * kf_f[None, :, :, :]
        y = (lambda x, s, axes=(-2,-1): jnp.fft.irfft2(x, s=s, axes=axes).astype(jnp.bfloat16))(y_f, (1, L), axes=(1, 2))[:, 0, :S, :]
        y = y + kv * ssm_D[None, None, :]
        return q * y

    def _B_ref(x, w_r, w_i):
        B, S, D = x.shape
        X = (lambda x, axes=(-2,-1): jnp.fft.rfft2(x.astype(jnp.float32), axes=axes))(x, axes=(-2, -1))
        W = w_r + 1j * w_i
        X = X * W
        y = (lambda x, s, axes=(-2,-1): jnp.fft.irfft2(x, s=s, axes=axes).astype(jnp.bfloat16))(X, (S, D), axes=(-2, -1))
        return y

    x = A_q
    g = _sigmoid((x * gate_w).sum(-1, keepdims=True))
    a = _A_ref(x, A_k, A_v, A_shift_k, A_ssm_k, A_ssm_D)
    b = _B_ref(x, B_w_r, B_w_i)
    return g * a + (1 - g) * b
```

```python
import numpy as np
import jax
import jax.numpy as jnp
from jax import lax
import jax.experimental.pallas as pl
import jax.experimental.pallas.tpu as pltpu

S, D = 2048, 1024
I32, F32, BF16 = jnp.int32, jnp.float32, jnp.bfloat16
RS = float(np.sqrt(0.5))


def _w(n, N):
    return np.exp(-2j * np.pi * (np.asarray(n) % N) / N)


def _pack_rows(m):
    u = np.asarray(m, np.float32).view(np.uint32).astype(np.uint64)
    b = ((u + 0x7FFF + ((u >> 16) & 1)) >> 16).astype(np.uint32)
    return np.ascontiguousarray(b[..., 0::2, :] | (b[..., 1::2, :] << 16)).view(np.int32)


def _make_consts():
    G = np.zeros((4, 256, 256))
    dl = np.arange(128)[:, None]
    j = np.arange(64)[None, :]
    for t in range(4):
        if t == 0:
            lo, hi = _w(dl * (8 * j), 1024), _w(dl * (4 + 8 * j), 1024)
            G[0, :128, 0:64], G[0, :128, 128:192] = lo.real, lo.imag
            G[0, 128:, 64:128], G[0, 128:, 192:256] = hi.real, hi.imag
        else:
            lo, hi = _w(dl * (t + 8 * j), 1024), _w(dl * (8 - t + 8 * j), 1024)
            G[t, :128, 0:64], G[t, :128, 128:192] = lo.real, lo.imag
            G[t, 128:, 0:64], G[t, 128:, 128:192] = -lo.imag, lo.real
            G[t, :128, 64:128], G[t, :128, 192:256] = hi.real, hi.imag
            G[t, 128:, 64:128], G[t, 128:, 192:256] = hi.imag, -hi.real
    M = np.zeros((4, 8, 128, 128))
    Mi = np.zeros((4, 8, 128, 128))
    km = np.arange(64)[:, None]
    sm = np.arange(64)[None, :]
    for kt in range(4):
        for sf in range(8):
            m = _w((8 * sm + sf) * (kt + 4 * km), 2048)
            M[kt, sf, :64, 0::2], M[kt, sf, :64, 1::2] = m.real, -m.imag
            M[kt, sf, 64:, 0::2], M[kt, sf, 64:, 1::2] = m.imag, m.real
            mi = np.conj(m).T * 2.0 ** -20
            Mi[kt, sf, :64, 0::2], Mi[kt, sf, :64, 1::2] = mi.real, -mi.imag
            Mi[kt, sf, 64:, 0::2], Mi[kt, sf, 64:, 1::2] = mi.imag, mi.real
    F = np.zeros((8, 256, 128))
    Fi = np.zeros((8, 128, 256))
    k1 = np.arange(128)[:, None]
    kr = np.arange(128)
    n1_of_k = 16 * (kr // 16) + 8 * (kr % 2) + (kr % 16) // 2
    for n2 in range(8):
        f = _w((8 * n1_of_k[None, :] + n2) * (4 * k1 + 1), 4096)
        F[n2, :128], F[n2, 128:] = f.real, f.imag
        fi = _w((8 * kr[None, :] + n2) * (4 * k1 + 1), 4096).T / 1024
        Fi[n2, :, 0::2], Fi[n2, :, 1::2] = fi.real, fi.imag
    jj = np.arange(256)
    cs = _w(jj[:, None] * jj[None, :], 256)
    CS = np.concatenate([cs.real, cs.imag], axis=1)
    tw = _w(np.arange(8)[:, None] * jj[None, :], 2048)
    f8 = _w(np.outer(np.arange(8), np.arange(8)), 8)
    misc = np.zeros((32, 256), np.float32)
    misc[0:8], misc[8:16] = tw.real, tw.imag
    misc[16:24, 0:8], misc[16:24, 8:16] = f8.real, -f8.imag
    misc[24:32, 0:8], misc[24:32, 8:16] = f8.imag, f8.real
    misc[16:24, 128:136], misc[16:24, 136:144] = f8.real, f8.imag
    misc[24:32, 128:136], misc[24:32, 136:144] = -f8.imag, f8.real
    return (_pack_rows(G), _pack_rows(M.reshape(32, 128, 128)), _pack_rows(Mi.reshape(32, 128, 128)),
            _pack_rows(F), _pack_rows(Fi), _pack_rows(CS), misc)


_CONSTS = _make_consts()


def _unpack(x, idx):
    return pltpu.unpack_elementwise(x, index=idx, packed_dtype=BF16, unpacked_dtype=F32)


def _pack(a, b):
    return pltpu.pack_elementwise([a, b], packed_dtype=BF16)


def _bf(x):
    return pltpu.bitcast(x, BF16)


def _dot(a, b):
    return lax.dot_general(a, b, (((1,), (0,)), ((), ())), preferred_element_type=F32)


def _dot_t(a, b):
    return lax.dot_general(a, b, (((1,), (1,)), ((), ())), preferred_element_type=F32)


def _rfft8(x):
    a0, a1, a2, a3 = x[0] + x[4], x[1] + x[5], x[2] + x[6], x[3] + x[7]
    b0, b1, nb2, b3 = x[0] - x[4], x[1] - x[5], x[6] - x[2], x[3] - x[7]
    e, o = a0 + a2, a1 + a3
    u, nv = (b1 - b3) * RS, (b1 + b3) * (-RS)
    return [(e + o, e - o), (b0 + u, nb2 + nv), (a0 - a2, a3 - a1), (b0 - u, nv - nb2)]


def _irfft8(T):
    (T0, T4), (T1r, T1i), (T2r, T2i), (T3r, T3i) = T
    a0, a1 = T0 + T4, T0 - T4
    p, q = a0 + T2r, a0 - T2r
    s, d = T1r + T3r, T1i - T3i
    u, v = T1r - T3r, T1i + T3i
    f, g = a1 - T2i, a1 + T2i
    x, y = (u - v) * RS, (u + v) * RS
    return [p + s, f + x, q - d, g - y, p - s, f - x, q + d, g + y]


def _fft4(r, i):
    ar, ai, br, bi = r[0] + r[2], i[0] + i[2], r[0] - r[2], i[0] - i[2]
    cr, ci, dr, di = r[1] + r[3], i[1] + i[3], r[1] - r[3], i[1] - i[3]
    return [ar + cr, br + di, ar - cr, br - di], [ai + ci, bi - dr, ai - ci, bi + dr]


def _ifft4(r, i):
    oi, orr = _fft4(i, r)
    return orr, oi


def _fft8(r, i):
    ar = [r[n] + r[n + 4] for n in range(4)]
    ai = [i[n] + i[n + 4] for n in range(4)]
    br = [r[n] - r[n + 4] for n in range(4)]
    bi = [i[n] - i[n + 4] for n in range(4)]
    er, ei = _fft4(ar, ai)
    ur, ui, vr, vi = br[1] - br[3], bi[1] - bi[3], br[1] + br[3], bi[1] + bi[3]
    pr, pi = (ur + vi) * RS, (ui - vr) * RS
    qr, qi = (vr + ui) * RS, (vi - ur) * RS
    sr, si = br[0] + bi[2], bi[0] - br[2]
    tr, ti = br[0] - bi[2], bi[0] + br[2]
    return ([er[0], sr + pr, er[1], tr + qi, er[2], sr - pr, er[3], tr - qi],
            [ei[0], si + pi, ei[1], ti - qr, ei[2], si - pi, ei[3], ti + qr])


def _ifft8(r, i):
    oi, orr = _fft8(i, r)
    return orr, oi


def _cmul(ar, ai, br, bi):
    return ar * br - ai * bi, ar * bi + ai * br


def _lanes(c):
    return slice(128 * c, 128 * c + 128)


NQ = 8


def _kernel(q_hbm, k_hbm, v_hbm, h_hbm, wr_hbm, wi_hbm, wrn_ref, win_ref, sk_ref, d_ref, gw_ref,
            G_hbm, M_hbm, Mi_hbm, F_hbm, Fi_hbm, CS_hbm, misc_ref,
            o_hbm,
            qb, kb, vb, hb, wb, ob, Gm, Mm, Mim, Fm, Fim, CSm,
            par, gate, gq, T0b, Tb, Z, U, Wf, V, Tc, Nq, bb, Xw, Gs, Yw,
            sem_q, sem_w, sem_a, sem_c, sem_o):
    QR = 256 // NQ

    def q_copy(n):
        return pltpu.make_async_copy(q_hbm.bitcast(I32).at[:, pl.ds(QR * n, QR), :],
                                     qb.at[:, pl.ds(QR * n, QR), :], sem_q.at[n])

    def w_copy(ri, a):
        src = (wr_hbm, wi_hbm)[ri]
        return pltpu.make_async_copy(src.at[pl.ds(0, 512), pl.ds(128 * a, 128)],
                                     wb.at[ri, a].bitcast(BF16), sem_w.at[ri, a])

    def a_copy(which, c):
        if which == 0:
            return pltpu.make_async_copy(k_hbm.bitcast(I32).at[:, pl.ds(128 * c, 128)],
                                         kb.at[c, pl.ds(8, 1024)], sem_a.at[0, c])
        if which == 1:
            return pltpu.make_async_copy(v_hbm.bitcast(I32).at[:, pl.ds(128 * c, 128)],
                                         vb.at[c], sem_a.at[1, c])
        return pltpu.make_async_copy(h_hbm.bitcast(I32).at[pl.ds(64 * c, 64), :],
                                     hb.at[c], sem_a.at[2, c])

    def c_copy(n):
        src = (G_hbm, M_hbm, Mi_hbm, F_hbm, Fi_hbm, CS_hbm)[n]
        dst = (Gm, Mm, Mim, Fm, Fim, CSm)[n]
        return pltpu.make_async_copy(src, dst, sem_c.at[n])

    def o_copy(c):
        return pltpu.make_async_copy(ob.at[c], o_hbm.bitcast(I32).at[:, pl.ds(128 * c, 128)], sem_o.at[c])

    q_copy(0).start()
    c_copy(0).start()
    for n in range(1, NQ):
        q_copy(n).start()
    c_copy(1).start()
    c_copy(5).start()
    for a in range(16):
        w_copy(0, a).start()
        w_copy(1, a).start()
    c_copy(2).start()
    c_copy(3).start()
    c_copy(4).start()
    for c in range(8):
        for which in range(3):
            a_copy(which, c).start()

    sk = sk_ref[...].astype(F32)
    for i in range(4):
        par[i] = jnp.broadcast_to(sk[i:i + 1, :], (8, D))
    par[4] = jnp.broadcast_to(d_ref[...].astype(F32).reshape(1, D), (8, D))
    par[5] = jnp.broadcast_to(gw_ref[...].astype(F32).reshape(1, D), (8, D))
    for c in range(8):
        kb[c, 0:8, :] = jnp.zeros((8, 128), I32)

    def p1(i, il):
        rows = pl.ds(pl.multiple_of(8 * i, 8), 8)
        for st in range(4):
            prow = pl.ds(pl.multiple_of(256 * st + 8 * i, 8), 8)
            xw = [qb[st, rows, _lanes(c)] for c in range(8)]
            for e in range(2):
                x = [_unpack(w, e) for w in xw]
                acc = x[0] * par[5, :, _lanes(0)]
                for c in range(1, 8):
                    acc = acc + x[c] * par[5, :, _lanes(c)]
                g = jnp.broadcast_to(jax.nn.sigmoid(jnp.sum(acc, axis=1, keepdims=True)), (8, 128))
                gate[e, prow, :] = 1.0 - g
                for c in range(8):
                    gq[c, e, prow, :] = x[c] * g
                T = _rfft8(x)
                T0b[e, prow, :] = T[0][0]
                r0 = 64 * il + 16 * st + 8 * e
                for t in range(4):
                    Tb[t, r0:r0 + 8, 0:128] = T[t][0]
                    Tb[t, r0:r0 + 8, 128:256] = T[t][1]

    NI = QR // 8

    def p2(i0, t):
        z = _dot(Tb[t], _bf(Gm[t]))
        for il in range(NI):
            rows = pl.ds(pl.multiple_of(8 * (i0 + il), 8), 8)
            for e in range(2):
                r = [z[64 * il + 16 * st + 8 * e:64 * il + 16 * st + 8 * e + 8, 0:128] for st in range(4)]
                im = [z[64 * il + 16 * st + 8 * e:64 * il + 16 * st + 8 * e + 8, 128:256] for st in range(4)]
                r, im = _fft4(r, im)
                for kt in range(4):
                    Z[t, kt, e, rows, :] = _pack(r[kt], im[kt])

    c_copy(0).wait()

    def phase1(n, carry):
        pltpu.make_async_copy(q_hbm.bitcast(I32).at[:, pl.ds(0, QR), :],
                              qb.at[:, pl.ds(0, QR), :], sem_q.at[n]).wait()
        for il in range(NI):
            p1(n * NI + il, il)
        for t in range(4):
            p2(n * NI, t)
        return carry

    with jax.named_scope("phase1"):
        lax.fori_loop(0, NQ, phase1, 0)

    def nyquist():
        sub = lax.broadcasted_iota(I32, (8, 128), 0)
        alt = (1 - 2 * (sub & 1)).astype(F32)
        R = []
        for jh in range(2):
            acc = jnp.zeros((8, 128), F32)
            for sf in range(8):
                tile = T0b[sf % 2, pl.ds(512 * jh + sf // 2, 128, stride=4), :].T
                s = tile[0:8]
                for n in range(1, 16):
                    s = s + tile[8 * n:8 * n + 8]
                s = jnp.sum(s * alt, axis=0, keepdims=True)
                acc = jnp.where(sub == sf, jnp.broadcast_to(s, (8, 128)), acc)
            R.append(acc)
        R = jnp.concatenate(R, axis=1)
        cs = _bf(CSm[...])
        A = _dot(R, cs)
        twr, twi = misc_ref[0:8, :], misc_ref[8:16, :]
        br, bi = _cmul(A[:, 0:256], A[:, 256:512], twr, twi)
        zpad = jnp.zeros((112, 256), F32)
        X = _dot(misc_ref[16:32, 0:128], jnp.concatenate([br, bi, zpad], axis=0))
        sub2 = lax.broadcasted_iota(I32, (8, 256), 0)
        wr = jnp.zeros((8, 256), F32)
        wi = jnp.zeros((8, 256), F32)
        for kf in range(8):
            cols = slice(256 * kf, 256 * kf + 256)
            wr = jnp.where(sub2 == kf, jnp.broadcast_to(wrn_ref[0:1, cols].astype(F32), (8, 256)), wr)
            wi = jnp.where(sub2 == kf, jnp.broadcast_to(win_ref[0:1, cols].astype(F32), (8, 256)), wi)
        yr, yi = _cmul(X[0:8], X[8:16], wr, wi)
        Y = _dot(misc_ref[16:32, 128:256], jnp.concatenate([yr, yi, zpad], axis=0))
        br, bi = _cmul(Y[0:8], Y[8:16], twr, -twi)
        z = _dot_t(jnp.concatenate([br, bi], axis=1), cs) * (0.5 * 2.0 ** -20)
        for sf in range(8):
            for jh in range(2):
                row = jnp.broadcast_to(z[sf:sf + 1, _lanes(jh)], (8, 128)) * alt
                Nq[sf, 128 * jh:128 * jh + 128, :] = jnp.concatenate([row] * 16, axis=0).T

    c_copy(5).wait()
    with jax.named_scope("nyq"):
        nyquist()

    def wprep(a, carry):
        sub = lax.broadcasted_iota(I32, (8, 128), 0)
        for ri in range(2):
            src = (wr_hbm, wi_hbm)[ri]
            pltpu.make_async_copy(src.at[pl.ds(0, 512), pl.ds(0, 128)],
                                  wb.at[ri, 0].bitcast(BF16), sem_w.at[ri, a]).wait()
        for ri in range(2):
            x = [wb[ri, a, pl.ds(m, 64, stride=4), :] for m in range(4)]
            ka = [_unpack(x[n // 2], n % 2) for n in range(8)]
            first = ka[0][0:8]
            ka[0] = jnp.concatenate([jnp.where(sub == 0, 0.5 * first, first), ka[0][8:]], axis=0)
            for t in range(4):
                tile = jnp.concatenate([ka[t], ka[8 - t if t else 4]], axis=0)
                Wf[ri, t, pl.ds(pl.multiple_of(128 * a, 128), 128), :] = tile.T
        return carry

    with jax.named_scope("wprep"):
        lax.fori_loop(0, 16, wprep, 0)

    def p3(t):
        for kt in range(4):
            for sf in range(8):
                x = Z[t, kt, sf % 2, pl.ds(sf // 2, 64, stride=4), :]
                U[kt, sf] = _dot(_bf(Mm[8 * kt + sf]), _bf(x))

    def p4(t):
        for kt in range(4):
            for g in range(8):
                r = [U[kt, sf, 8 * g:8 * g + 8, :] for sf in range(8)]
                im = [U[kt, sf, 64 + 8 * g:64 + 8 * g + 8, :] for sf in range(8)]
                r, im = _fft8(r, im)
                for kf in range(8):
                    rows = pl.ds(256 * kf + 32 * g + kt, 8, stride=4)
                    r[kf], im[kf] = _cmul(r[kf], im[kf], Wf[0, t, rows, :], Wf[1, t, rows, :])
                r, im = _ifft8(r, im)
                for sf in range(8):
                    V[kt, sf, 8 * g:8 * g + 8, :] = _pack(r[sf], im[sf])

    def p56(t):
        for sf in range(8):
            o = [_dot(_bf(Mim[8 * kt + sf]), _bf(V[kt, sf])) for kt in range(4)]
            r, im = _ifft4([x[0:64] for x in o], [x[64:128] for x in o])
            lhs = jnp.concatenate([jnp.concatenate(r, axis=0), jnp.concatenate(im, axis=0)], axis=1)
            Tc[t, sf] = _dot_t(lhs, _bf(Gm[t]))

    c_copy(1).wait()
    c_copy(2).wait()

    def phase2(t, carry):
        p3(t)
        p4(t)
        p56(t)
        return carry

    with jax.named_scope("phase2"):
        lax.fori_loop(0, 4, phase2, 0)

    def p7(sf, carry):
        for n in range(32):
            rows = slice(8 * n, 8 * n + 8)
            T = [(Tc[t, sf, rows, 0:128], Tc[t, sf, rows, 128:256]) for t in range(4)]
            T[0] = (T[0][0] + Nq[sf, rows, :], T[0][1])
            b = _irfft8(T)
            omg = gate[sf % 2, pl.ds(32 * n + sf // 2, 8, stride=4), :]
            for c in range(8):
                bb[c, sf, rows, :] = b[c] * omg
        return carry

    with jax.named_scope("p7"):
        lax.fori_loop(0, 8, p7, 0)

    def a1(c):
        cf = [par[i, :, pl.ds(pl.multiple_of(128 * c, 128), 128)] for i in range(4)]
        for r in range(2):
            for G in range(8):
                kv = []
                for gh in range(2):
                    j0 = 128 * r + 16 * G + 8 * gh
                    kw = [kb[c, pl.ds(8 + 4 * j0 + m, 8, stride=4), :] for m in range(4)]
                    kp = [kb[c, pl.ds(4 + 4 * j0 + m, 8, stride=4), :] for m in (2, 3)]
                    vw = [vb[c, pl.ds(4 * j0 + m, 8, stride=4), :] for m in range(4)]
                    kk = [_unpack(kp[0], 1), _unpack(kp[1], 0), _unpack(kp[1], 1)]
                    kk += [_unpack(kw[n // 2], n % 2) for n in range(8)]
                    out = []
                    for n in range(8):
                        s = (kk[n + 3] * cf[0] + kk[n + 2] * cf[1]) + (kk[n + 1] * cf[2] + kk[n] * cf[3])
                        out.append(s * _unpack(vw[n // 2], n % 2))
                    kv.append(out)
                for n in range(8):
                    Xw[n, 8 * G:8 * G + 8, _lanes(r)] = _pack(kv[0][n], kv[1][n])

    def a2(c):
        lane = lax.broadcasted_iota(I32, (8, 128), 1)
        idx = 64 * (lane & 1) + 8 * ((lane >> 1) & 7) + (lane >> 4)
        for a in range(16):
            x = jnp.concatenate([jnp.take_along_axis(hb[c, 8 * n:8 * n + 8, _lanes(a)], idx, axis=1)
                                 for n in range(8)], axis=0)
            y = pltpu.bitcast(_bf(x).T, I32)
            for n in range(8):
                Xw[n, 8 * (a % 8):8 * (a % 8) + 8, _lanes(2 + a // 8)] = y[8 * n:8 * n + 8]

    def a3():
        for n in range(8):
            Gs[n] = _dot(_bf(Fm[n]), _bf(Xw[n]))

    def a4(c):
        dv = par[4, :, pl.ds(pl.multiple_of(128 * c, 128), 128)]
        for g in range(16):
            def load(s):
                return ([Gs[n, 8 * g:8 * g + 8, _lanes(s)] for n in range(8)],
                        [Gs[n, 128 + 8 * g:128 + 8 * g + 8, _lanes(s)] for n in range(8)])
            x0r, x0i = _fft8(*load(0))
            h1r, h1i = _fft8(*load(3))
            p = [_cmul(h1r[n], h1i[n], x0r[n], x0i[n]) for n in range(8)]
            hr, hi = load(2)
            hr[0] = hr[0] + dv
            h0r, h0i = _fft8(hr, hi)
            y0 = [_cmul(h0r[n], h0i[n], x0r[n], x0i[n]) for n in range(8)]
            p = [(p[n][0] - y0[n][1], p[n][1] + y0[n][0]) for n in range(8)]
            r, im = _ifft8([y[0] for y in y0], [y[1] for y in y0])
            for n in range(8):
                Yw[n, 8 * g:8 * g + 8, 0:128] = _pack(r[n], im[n])
            x1r, x1i = _fft8(*load(1))
            y1 = [_cmul(h0r[n], h0i[n], x1r[n], x1i[n]) for n in range(8)]
            r, im = _ifft8([y1[n][0] + p[n][0] for n in range(8)], [y1[n][1] + p[n][1] for n in range(8)])
            for n in range(8):
                Yw[n, 8 * g:8 * g + 8, 128:256] = _pack(r[n], im[n])

    def a5(c):
        for m in range(4):
            y = [_dot(_bf(Fim[2 * m + e]), _bf(Yw[2 * m + e])) for e in range(2)]
            for r in range(2):
                rows = pl.ds(512 * r + m, 128, stride=4)
                o = [gq[c, e, rows, :] * y[e][:, _lanes(r)] + bb[c, 2 * m + e, 128 * r:128 * r + 128, :]
                     for e in range(2)]
                ob[c, rows, :] = _pack(o[0], o[1])

    c_copy(3).wait()
    c_copy(4).wait()

    def phase3(c, carry):
        pltpu.make_async_copy(k_hbm.bitcast(I32).at[:, pl.ds(0, 128)], vb.at[0], sem_a.at[0, c]).wait()
        pltpu.make_async_copy(k_hbm.bitcast(I32).at[:, pl.ds(0, 128)], vb.at[0], sem_a.at[1, c]).wait()
        pltpu.make_async_copy(h_hbm.bitcast(I32).at[pl.ds(0, 64), :], hb.at[0], sem_a.at[2, c]).wait()
        a1(c)
        a2(c)
        a3()
        a4(c)
        a5(c)
        pltpu.make_async_copy(ob.at[c], o_hbm.bitcast(I32).at[:, pl.ds(pl.multiple_of(128 * c, 128), 128)],
                              sem_o.at[c]).start()
        return carry

    with jax.named_scope("phase3"):
        lax.fori_loop(0, 8, phase3, 0)
    for c in range(8):
        o_copy(c).wait()


@jax.jit
def pallas_gated_mix__ssm_conv_h3__spectral_gfnet__prompt_kernel(A_q, A_k, A_v, A_shift_k, A_ssm_k, A_ssm_D, B_x, B_w_r, B_w_i, gate_w):
    del B_x
    wr_t, wi_t = B_w_r.T, B_w_i.T
    any_spec = pl.BlockSpec(memory_space=pl.ANY)
    V = pltpu.VMEM
    out = pl.pallas_call(
        _kernel,
        grid=(1,),
        in_specs=[any_spec] * 6 + [
            pl.BlockSpec((16, 2048), lambda i: (32, 0)),
            pl.BlockSpec((16, 2048), lambda i: (32, 0)),
            pl.BlockSpec((4, D), lambda i: (0, 0)),
            pl.BlockSpec((D,), lambda i: (0,)),
            pl.BlockSpec((D,), lambda i: (0,)),
        ] + [any_spec] * 6 + [pl.BlockSpec((32, 256), lambda i: (0, 0))],
        out_specs=any_spec,
        out_shape=jax.ShapeDtypeStruct((S, D), BF16),
        scratch_shapes=[
            V((4, 256, D), I32), V((8, 1032, 128), I32), V((8, 1024, 128), I32), V((8, 64, S), I32),
            V((2, 16, 256, 128), I32), V((8, 1024, 128), I32),
            V((4, 128, 256), I32), V((32, 64, 128), I32), V((32, 64, 128), I32),
            V((8, 128, 128), I32), V((8, 64, 256), I32), V((128, 512), I32),
            V((6, 8, D), F32), V((2, 1024, 128), F32), V((8, 2, 1024, 128), F32), V((2, 1024, 128), F32),
            V((4, 2048 // NQ, 256), F32), V((4, 4, 2, 256, 128), I32), V((4, 8, 128, 128), F32),
            V((2, 4, S, 128), F32), V((4, 8, 64, 128), I32), V((4, 8, 256, 256), F32),
            V((8, 256, 128), F32), V((8, 8, 256, 128), F32),
            V((8, 64, 512), I32), V((8, 256, 512), F32), V((8, 128, 256), I32),
            pltpu.SemaphoreType.DMA((NQ,)), pltpu.SemaphoreType.DMA((2, 16)),
            pltpu.SemaphoreType.DMA((3, 8)), pltpu.SemaphoreType.DMA((6,)), pltpu.SemaphoreType.DMA((8,)),
        ],
        compiler_params=pltpu.CompilerParams(vmem_limit_bytes=120 * 2 ** 20),
        name="gated_mix",
    )(A_q.reshape(4, 512, D), A_k.reshape(S, D), A_v.reshape(S, D), A_ssm_k, wr_t, wi_t, wr_t, wi_t,
      A_shift_k.T, A_ssm_D, gate_w, *_CONSTS)
    return out.reshape(1, S, D)
```

```python
import numpy as np
import jax
import jax.numpy as jnp
from jax import lax
import jax.experimental.pallas as pl
import jax.experimental.pallas.tpu as pltpu

S, D = 2048, 1024
I32, F32, BF16 = jnp.int32, jnp.float32, jnp.bfloat16
RS = float(np.sqrt(0.5))
SIGN2 = int(np.array(0x80008000, np.uint32).view(np.int32))

OPT = dict(m3=64, m5=32, m2=128, m6=64, mp3=128, mp5=128, nq=8, even=1, nl3=256, sched=0, nx=3, lag=0.02, look=0, dense0=0, cond=1)

def _w(n, N):
    return np.exp(-2j * np.pi * (np.asarray(n) % N) / N)


def _pack_rows(m):
    u = np.asarray(m, np.float32).view(np.uint32).astype(np.uint64)
    b = ((u + 0x7FFF + ((u >> 16) & 1)) >> 16).astype(np.uint32)
    return np.ascontiguousarray(b[..., 0::2, :] | (b[..., 1::2, :] << 16)).view(np.int32)


def _tile_kd(t):
    kd = np.zeros(128, np.int64)
    for lane in range(128):
        i2, r = lane // 8, lane % 8
        e = t % 2
        own = (r % 2 == 0) if e == 0 else (r % 4 in (0, 3))
        if own == (t < 2):
            i, rr = 2 * i2, r
        else:
            i, rr = 2 * i2 + 1, (r - (1 + e)) % 8
        kd[lane] = 16 * i + 8 * (rr // 4) + 2 * (rr % 4) + e
    return kd


def _make_consts():
    G = np.zeros((4, 128, 256))
    lo = np.zeros((4, 128), np.int32)
    dl = np.arange(128)[:, None]
    for t in range(4):
        kd = _tile_kd(t)
        g = _w(dl * kd[None, :], 1024)
        G[t, :, :128], G[t, :, 128:] = g.real, g.imag
        lo[t] = kd % 8 == t
    Gi = np.zeros((11, 128, 128))
    for t in range(4):
        g = _w(dl * _tile_kd(t)[None, :], 1024).T
        own = lo[t][:, None] == 1
        if t == 0:
            Gi[0] = np.where(own, g.real, np.roll(g.imag, 2, axis=0))
            Gi[1] = np.where(own, np.roll(g.real, -2, axis=0), g.imag)
        else:
            al, be = np.where(own, g.real, g.imag), np.where(own, g.imag, g.real)
            Gi[3 * t - 1], Gi[3 * t], Gi[3 * t + 1] = al, be - al, al + be
    M = np.zeros((4, 64, 128), np.float32)
    sm = np.concatenate([np.arange(0, 64, 2), np.arange(1, 64, 2)])[:, None]
    km = np.arange(128)[None, :] // 2
    d64 = np.conj(_w(sm * km, 64) * np.where(np.arange(128) % 2 == 0, 1, -1j)[None, :])
    M[0], M[1] = d64.real, d64.imag
    for kt in range(4):
        al = np.conj(_w(sm[:, 0] * kt, 256))
        M[2, :, 2 * kt], M[2, :, 2 * kt + 1] = al.real, al.imag
        for sf in range(8):
            be = np.conj(_w(sf * (kt + 4 * km[0]), 2048))
            M[3, 2 * (8 * kt + sf)], M[3, 2 * (8 * kt + sf) + 1] = be.real, be.imag
    F = np.zeros((8, 256, 128))
    Fi = np.zeros((8, 128, 256))
    k1 = np.arange(128)[:, None]
    kr = np.arange(128)
    n1_of_k = 16 * (kr // 16) + 8 * (kr % 2) + (kr % 16) // 2
    for n2 in range(8):
        f = _w((8 * n1_of_k[None, :] + n2) * (4 * k1 + 1), 4096)
        F[n2, :128], F[n2, 128:] = f.real, f.imag
        fi = _w((8 * kr[None, :] + n2) * (4 * k1 + 1), 4096).T / 1024
        Fi[n2, :, 0::2], Fi[n2, :, 1::2] = fi.real, fi.imag
    jj = np.arange(256)
    cs = _w(jj[:, None] * jj[None, :], 256)
    CS = np.concatenate([cs.real, cs.imag], axis=1)
    tw = _w(np.arange(8)[:, None] * jj[None, :], 2048)
    f8 = _w(np.outer(np.arange(8), np.arange(8)), 8)
    misc = np.zeros((32, 256), np.float32)
    misc[0:8], misc[8:16] = tw.real, tw.imag
    misc[16:24, 0:8], misc[16:24, 8:16] = f8.real, -f8.imag
    misc[24:32, 0:8], misc[24:32, 8:16] = f8.imag, f8.real
    misc[16:24, 128:136], misc[16:24, 136:144] = f8.real, f8.imag
    misc[24:32, 128:136], misc[24:32, 136:144] = -f8.imag, f8.real
    consts = (_pack_rows(G), M,
              _pack_rows(F), _pack_rows(Fi), _pack_rows(CS), misc, _pack_rows(Gi))
    return consts, lo


_CONSTS, _LO = _make_consts()
assert np.array_equal(_LO, np.tile(_LO[:, :8], 16))


def _unpack(x, idx):
    return pltpu.unpack_elementwise(x, index=idx, packed_dtype=BF16, unpacked_dtype=F32)


def _pack(a, b):
    return pltpu.bitcast(pltpu.pack_elementwise([a, b], packed_dtype=BF16), I32)


def _bf(x):
    return pltpu.bitcast(x, BF16)


def _dot(a, b):
    return lax.dot_general(a, b, (((1,), (0,)), ((), ())), preferred_element_type=F32)


def _dot_t(a, b):
    return lax.dot_general(a, b, (((1,), (1,)), ((), ())), preferred_element_type=F32)


def _rfft8(x):
    a0, a1, a2, a3 = x[0] + x[4], x[1] + x[5], x[2] + x[6], x[3] + x[7]
    b0, b1, nb2, b3 = x[0] - x[4], x[1] - x[5], x[6] - x[2], x[3] - x[7]
    e, o = a0 + a2, a1 + a3
    u, nv = (b1 - b3) * RS, (b1 + b3) * (-RS)
    return [(e + o, e - o), (b0 + u, nb2 + nv), (a0 - a2, a3 - a1), (b0 - u, nv - nb2)]


def _irfft8(T):
    (T0, T4), (T1r, T1i), (T2r, T2i), (T3r, T3i) = T
    a0, a1 = T0 + T4, T0 - T4
    p, q = a0 + T2r, a0 - T2r
    s, d = T1r + T3r, T1i - T3i
    u, v = T1r - T3r, T1i + T3i
    f, g = a1 - T2i, a1 + T2i
    x, y = (u - v) * RS, (u + v) * RS
    return [p + s, f + x, q - d, g - y, p - s, f - x, q + d, g + y]


def _fft4(r, i):
    ar, ai, br, bi = r[0] + r[2], i[0] + i[2], r[0] - r[2], i[0] - i[2]
    cr, ci, dr, di = r[1] + r[3], i[1] + i[3], r[1] - r[3], i[1] - i[3]
    return [ar + cr, br + di, ar - cr, br - di], [ai + ci, bi - dr, ai - ci, bi + dr]


def _ifft4(r, i):
    oi, orr = _fft4(i, r)
    return orr, oi


def _fft4o(br, bi):
    ur, ui, vr, vi = br[1] - br[3], bi[1] - bi[3], br[1] + br[3], bi[1] + bi[3]
    pr, pi = (ur + vi) * RS, (ui - vr) * RS
    qr, qi = (vr + ui) * RS, (vi - ur) * RS
    sr, si = br[0] + bi[2], bi[0] - br[2]
    tr, ti = br[0] - bi[2], bi[0] + br[2]
    return [sr + pr, tr + qi, sr - pr, tr - qi], [si + pi, ti - qr, si - pi, ti + qr]


def _ifft4o(xr, xi):
    sr, si, pr, pi = xr[0] + xr[2], xi[0] + xi[2], xr[0] - xr[2], xi[0] - xi[2]
    tr, ti, qi, qr = xr[1] + xr[3], xi[1] + xi[3], xr[1] - xr[3], xi[3] - xi[1]
    ur, ui, vr, vi = pr - qi, pi + qr, qr - pi, pr + qi
    return ([sr + tr, (ur + vr) * RS, ti - si, (vr - ur) * RS],
            [si + ti, (ui + vi) * RS, sr - tr, (vi - ui) * RS])


def _fft8(r, i):
    er, ei = _fft4([r[n] + r[n + 4] for n in range(4)], [i[n] + i[n + 4] for n in range(4)])
    orr, oi = _fft4o([r[n] - r[n + 4] for n in range(4)], [i[n] - i[n + 4] for n in range(4)])
    return [x for p in zip(er, orr) for x in p], [x for p in zip(ei, oi) for x in p]


def _ifft8(r, i):
    oi, orr = _fft8(i, r)
    return orr, oi


def _cmul(ar, ai, br, bi):
    return ar * br - ai * bi, ar * bi + ai * br


def _lanes(c):
    return slice(128 * c, 128 * c + 128)


def _rows8(start):
    if isinstance(start, int):
        return slice(start, start + 8)
    return pl.ds(pl.multiple_of(start, 8), 8)


def _span(n, size):
    return pl.ds(size * n if isinstance(n, int) else pl.multiple_of(size * n, size), size)


def _mix(*streams):
    live = [list(g) if isinstance(g, tuple) else [g, 0.0] for g in streams]
    n = len(live)
    while live:
        cur = min(live, key=lambda z: z[1])
        try:
            f = next(cur[0])
        except StopIteration:
            live.remove(cur)
            continue
        cur[1] += f
        yield f / n


def _chain(*parts):
    total = float(sum(w for _, w in parts))
    for g, w in parts:
        for f in g:
            yield f * w / total


def _kernel(q_hbm, k_hbm, v_hbm, h_hbm, wr_hbm, wi_hbm, sk_hbm, d_hbm, gw_hbm,
            G_hbm, M_hbm, F_hbm, Fi_hbm, CS_hbm, misc_hbm, Gi_hbm,
            o_hbm,
            qb, kb, vb, hb, wb, ob, Gm, Mt, Mm, Mim, Fm, Fim, CSm, misc, Gim, skb, db, gwb, wn,
            par, pc, gate, gq, T0b, Tw0, Tw1, Zn, U, Wf0, Wf1, V0, V1, Tc, Nq, bb,
            Xx, Xh0, Xh1, Gs0, Gs1, Yw0, Yw1,
            sem_q, sem_w, sem_a, sem_c, sem_o):
    NQ = OPT["nq"]
    QR = 256 // NQ
    NI = QR // 8
    NX = OPT["nx"]
    Tw, Wf, V = (Tw0, Tw1), (Wf0, Wf1), (V0, V1)
    Xh, Gs, Yw = (Xh0, Xh1), (Gs0, Gs1), (Yw0, Yw1)

    def q_copies(n):
        rows = _span(n, QR)
        return [pltpu.make_async_copy(q_hbm.bitcast(I32).at[pl.ds(2 * h, 2), rows, :],
                                      qb.at[pl.ds(2 * h, 2), rows, :], sem_q.at[n, h]) for h in range(2)]

    def q_start(n):
        for c in q_copies(n):
            c.start()

    def q_wait(n):
        for c in q_copies(n):
            c.wait()

    def w_copy(ri):
        return pltpu.make_async_copy((wr_hbm, wi_hbm)[ri].at[pl.ds(0, 512), :], wb.at[ri].bitcast(BF16), sem_w.at[ri])

    def a_copy(which, c):
        if which == 0:
            return pltpu.make_async_copy(k_hbm.bitcast(I32).at[:, _span(c, 128)],
                                         kb.at[c, pl.ds(8, 1024)], sem_a.at[0, c])
        if which == 1:
            return pltpu.make_async_copy(v_hbm.bitcast(I32).at[:, _span(c, 128)], vb.at[c], sem_a.at[1, c])
        return pltpu.make_async_copy(h_hbm.bitcast(I32).at[_span(c, 64), :], hb.at[c], sem_a.at[2, c])

    c_pairs = dict(G=(G_hbm, Gm.at[:, pl.ds(0, 64), :]), M=(M_hbm, Mt),
                   Gi=(Gi_hbm, Gim), F=(F_hbm, Fm), Fi=(Fi_hbm, Fim),
                   CS=(CS_hbm, CSm), misc=(misc_hbm, misc), sk=(sk_hbm, skb), d=(d_hbm, db), gw=(gw_hbm, gwb),
                   wnr=(wr_hbm.at[pl.ds(512, 1), :], wn.at[0]), wni=(wi_hbm.at[pl.ds(512, 1), :], wn.at[1]))
    c_names = list(c_pairs)

    def c_copy(name):
        src, dst = c_pairs[name]
        return pltpu.make_async_copy(src, dst, sem_c.at[c_names.index(name)])

    def o_copy(c, slot):
        return pltpu.make_async_copy(ob.at[slot], o_hbm.bitcast(I32).at[:, _span(c, 128)], sem_o.at[c])

    def own_lanes(t):
        lane = lax.broadcasted_iota(I32, (8, 128), 1)
        bits = int(sum(int(b) << n for n, b in enumerate(_LO[t][:8])))
        return ((bits >> (lane & 7)) & 1) == 1

    def expand_g():
        for t in range(4):
            lo = own_lanes(t)
            for n in range(8):
                top, bot = slice(8 * n, 8 * n + 8), slice(64 + 8 * n, 72 + 8 * n)
                gr, gi = Gm[t, top, 0:128], Gm[t, top, 128:256]
                if t == 0:
                    Gm[t, top, 0:128], Gm[t, top, 128:256] = jnp.where(lo, gr, 0), jnp.where(lo, gi, 0)
                    Gm[t, bot, 0:128], Gm[t, bot, 128:256] = jnp.where(lo, 0, gr), jnp.where(lo, 0, gi)
                else:
                    Gm[t, bot, 0:128] = gi ^ jnp.where(lo, SIGN2, 0)
                    Gm[t, bot, 128:256] = gr ^ jnp.where(lo, 0, SIGN2)
        yield 1.0

    def make_m():
        for kt in range(4):
            base = []
            for r in range(8):
                dr, di = Mt[0, 8 * r:8 * r + 8, :], Mt[1, 8 * r:8 * r + 8, :]
                if kt:
                    col = Mt[2, 8 * r:8 * r + 8, :]
                    ar = jnp.take_along_axis(col, jnp.full((8, 128), 2 * kt, I32), axis=1)
                    ai = jnp.take_along_axis(col, jnp.full((8, 128), 2 * kt + 1, I32), axis=1)
                    dr, di = _cmul(dr, di, ar, ai)
                base.append((dr, di))
            for sf in range(8):
                n = 8 * kt + sf
                br = jnp.broadcast_to(Mt[3, 2 * n:2 * n + 1, :], (8, 128))
                bi = jnp.broadcast_to(Mt[3, 2 * n + 1:2 * n + 2, :], (8, 128))
                rows = []
                for b in range(4):
                    er, ei = _cmul(*base[b], br, bi)
                    orr, oi = _cmul(*base[4 + b], br, bi)
                    rows += [_pack(er, orr), _pack(ei, oi)]
                    Mm[n, pl.ds(16 * b, 8, stride=2), :] = _pack(er, ei)
                    Mm[n, pl.ds(16 * b + 1, 8, stride=2), :] = _pack(orr, oi)
                for r in range(8):
                    Mim[n, 8 * r:8 * r + 8, :] = rows[r]
                yield 1.0 / 32

    def flip_m():
        for n in range(32):
            Mm[n] = pltpu.bitcast(_bf(Mm[n]).T, I32)
            yield 1.0 / 32

    def p1(n, slot):
        for il in range(NI):
            i = n * NI + il
            for st in range(4):
                prow = _rows8(256 * st + 8 * i)
                xw = [qb[st, _rows8(8 * i), _lanes(c)] for c in range(8)]
                Ts = []
                for e in range(2):
                    x = [_unpack(w, e) for w in xw]
                    pr = [x[c] * par[0, :, _lanes(c)] for c in range(8)]
                    acc = ((pr[0] + pr[1]) + (pr[2] + pr[3])) + ((pr[4] + pr[5]) + (pr[6] + pr[7]))
                    th = 0.5 * jnp.tanh(0.5 * jnp.broadcast_to(jnp.sum(acc, axis=1, keepdims=True), (8, 128)))
                    g = 0.5 + th
                    gate[e, prow, :] = (0.5 - th) * 2.0 ** -20
                    for c in range(8):
                        gq[c, e, prow, :] = x[c] * g
                    Ts.append(_rfft8(x))
                    T0b[e, prow, :] = Ts[e][0][0]
                    yield 1.0 / (8 * NI)
                r0 = 32 * il + 8 * st
                for t in range(4):
                    for h in range(2):
                        Tw[slot][t, r0:r0 + 8, _lanes(h)] = _pack(Ts[0][t][h], Ts[1][t][h])

    def p2(n, slot):
        m2 = OPT["m2"]
        for t in range(4):
            for part in range(64 * NI // m2):
                z = _dot(_bf(Tw[slot][t, m2 // 2 * part:m2 // 2 * (part + 1), :]), _bf(Gm[t]))
                for ii in range(m2 // 64):
                    i = n * NI + part * (m2 // 64) + ii
                    for u in range(2):
                        rows = [slice(64 * ii + 16 * st + 8 * u, 64 * ii + 16 * st + 8 * u + 8) for st in range(4)]
                        r, im = _fft4([z[s, 0:128] for s in rows], [z[s, 128:256] for s in rows])
                        for kt in range(4):
                            Zn[t, kt, _rows8(16 * i + 8 * u), :] = _pack(r[kt], im[kt])
                yield m2 / (256.0 * NI)

    def p3(t):
        mp = OPT["mp3"]
        for kt in range(4):
            for sf in range(8):
                x = _bf(Zn[t, kt, pl.ds(sf, 64, stride=8), :])
                for h in range(128 // mp):
                    U[t, kt, sf, mp * h:mp * h + mp, :] = _dot(
                        _bf(Mm[8 * kt + sf, mp // 2 * h:mp // 2 * (h + 1), :]), x)
                if sf % 4 == 3:
                    yield 1.0 / 8

    def p4a(t):
        for kt in range(4):
            for g in range(8):
                re, im = pl.ds(16 * g, 8, stride=2), pl.ds(16 * g + 1, 8, stride=2)
                r, i = _fft8([U[t, kt, sf, re, :] for sf in range(8)], [U[t, kt, sf, im, :] for sf in range(8)])
                for kf in range(8):
                    U[t, kt, kf, 16 * g:16 * g + 8, :] = r[kf]
                    U[t, kt, kf, 16 * g + 8:16 * g + 16, :] = i[kf]
                yield 1.0 / 32

    def wprep(t, p):
        e = t % 2
        sub = lax.broadcasted_iota(I32, (8, 128), 0)
        own = ((sub & 1) == 0) if e == 0 else (((sub + 1) & 2) == 0)
        for a in list(range(0, 16, 2)) + list(range(1, 16, 2)):
            rows = []
            for i2 in range(16):
                x = []
                for ri in range(2):
                    A = wb[ri, 16 * i2:16 * i2 + 8, _lanes(a)]
                    B = pltpu.roll(wb[ri, 16 * i2 + 8:16 * i2 + 16, _lanes(a)], 1 + e, 0)
                    x.append(jnp.where(own, A, B) if t < 2 else jnp.where(own, B, A))
                if t == 0 and i2 == 0:
                    half = jnp.where(sub == 0, 0.5, 1.0)
                    rows.append(_pack(_unpack(x[0], e) * half, _unpack(x[1], e) * half))
                elif e == 0:
                    rows.append(pltpu.bitcast(pltpu.pack_elementwise(x, packed_dtype=jnp.int16), I32))
                else:
                    rows.append(_pack(_unpack(x[0], e), _unpack(x[1], e)))
            Wf[p][128 * a:128 * a + 128, :] = jnp.concatenate(rows, axis=0).T
            yield 1.0 / 16

    def p4b(t, p, full=False):
        w, v = Wf[p], V[p]
        u = 1.0 / (32 * (3 if full else 2))
        for g in range(8):
            for kt in range(4):
                if full:
                    re, ie = pl.ds(16 * g, 8, stride=2), pl.ds(16 * g + 1, 8, stride=2)
                else:
                    re, ie = slice(16 * g, 16 * g + 8), slice(16 * g + 8, 16 * g + 16)
                r = [U[t, kt, n, re, :] for n in range(8)]
                im = [U[t, kt, n, ie, :] for n in range(8)]
                if full:
                    r, im = _fft8(r, im)
                    yield u
                for kf in range(8):
                    ww = w[pl.ds(256 * kf + 32 * g + kt, 8, stride=4), :]
                    r[kf], im[kf] = _cmul(r[kf], im[kf], _unpack(ww, 0), _unpack(ww, 1))
                yield u
                r, im = _ifft8(r, im)
                for sf in range(8):
                    v[kt, sf, 8 * g:8 * g + 8, :] = _pack(r[sf], im[sf])
                yield u

    def p567(t, p, mp=64, m6=32, look=1):
        lo = own_lanes(t)
        cost6 = 2.0 if t == 0 else 3.0
        total = 8 * (128 + 64 * cost6)

        def first(sf, h):
            o = [_dot(_bf(Mim[8 * kt + sf, mp // 2 * h:mp // 2 * (h + 1), :]), _bf(V[p][kt, sf]))
                 for kt in range(4)]
            la, lb, dest = [], [], []
            for b in range(mp // 32):
                for u in range(2):
                    r, im = _ifft4([x[32 * b + 8 * u:32 * b + 8 * u + 8] for x in o],
                                   [x[32 * b + 16 + 8 * u:32 * b + 16 + 8 * u + 8] for x in o])
                    for st in range(4):
                        if t == 0:
                            la.append(jnp.where(lo, r[st], pltpu.roll(im[st], 2, 1)))
                            lb.append(jnp.where(lo, pltpu.roll(r[st], 126, 1), im[st]))
                        else:
                            la.append(jnp.where(lo, r[st], im[st]))
                            lb.append(jnp.where(lo, im[st], r[st]))
                        dest.append(64 * st + 16 * (h * (mp // 32) + b) + 8 * u)
            return sf, la, lb, dest

        def second(sf, la, lb, dest):
            for part in range(len(la) * 8 // m6):
                sel = slice(part * m6 // 8, (part + 1) * m6 // 8)
                xa, xb = jnp.concatenate(la[sel], axis=0), jnp.concatenate(lb[sel], axis=0)
                if t == 0:
                    yr, yi = _dot(xa, _bf(Gim[0])), _dot(xb, _bf(Gim[1]))
                else:
                    yp = _dot(xa + xb, _bf(Gim[3 * t - 1]))
                    yq = _dot(xb, _bf(Gim[3 * t]))
                    ys = _dot(xa, _bf(Gim[3 * t + 1]))
                for n, j0 in enumerate(dest[sel]):
                    r8 = slice(8 * n, 8 * n + 8)
                    tr, ti = (yr[r8], yi[r8]) if t == 0 else (yp[r8] + yq[r8], yp[r8] - ys[r8])
                    rows = slice(j0, j0 + 8)
                    if t > 0:
                        Tc[t - 1, sf, rows, 0:128] = tr
                        Tc[t - 1, sf, rows, 128:256] = ti
                    else:
                        T = [(Tc[tt, sf, rows, 0:128], Tc[tt, sf, rows, 128:256]) for tt in range(3)]
                        b_ = _irfft8([(tr + Nq[sf, rows, :], ti)] + T)
                        omg = gate[sf % 2, pl.ds(4 * j0 + sf // 2, 8, stride=4), :]
                        for c in range(8):
                            bb[c, sf, rows, :] = b_[c] * omg
                yield (mp * m6 / (len(la) * 8) + m6 * cost6 / 4) / total

        pend = []
        for sf in range(8):
            for h in range(128 // mp):
                pend.append(first(sf, h))
                if len(pend) > look:
                    yield from second(*pend.pop(0))
        while pend:
            yield from second(*pend.pop(0))

    def nyq_fwd():
        sub = lax.broadcasted_iota(I32, (8, 128), 0)
        alt = (1 - 2 * (sub & 1)).astype(F32)
        for jh in range(2):
            acc = jnp.zeros((8, 128), F32)
            for sf in range(8):
                tile = T0b[sf % 2, pl.ds(512 * jh + sf // 2, 128, stride=4), :].T
                s = tile[0:8]
                for n in range(1, 16):
                    s = s + tile[8 * n:8 * n + 8]
                s = jnp.sum(s * alt, axis=0, keepdims=True)
                acc = jnp.where(sub == sf, jnp.broadcast_to(s, (8, 128)), acc)
                yield 1.0 / 16
            par[1, :, _lanes(jh)] = acc

    def nyq_rest():
        sub = lax.broadcasted_iota(I32, (8, 128), 0)
        alt = (1 - 2 * (sub & 1)).astype(F32)
        A = _dot(par[1, :, 0:256], _bf(CSm[...]))
        twr, twi = misc[0:8, :], misc[8:16, :]
        br, bi = _cmul(A[:, 0:256], A[:, 256:512], twr, twi)
        yield 0.1
        zpad = jnp.zeros((112, 256), F32)
        X = _dot(misc[16:32, 0:128], jnp.concatenate([br, bi, zpad], axis=0))
        sub2 = lax.broadcasted_iota(I32, (8, 256), 0)
        wr = jnp.zeros((8, 256), F32)
        wi = jnp.zeros((8, 256), F32)
        for kf in range(8):
            cols = slice(256 * kf, 256 * kf + 256)
            wr = jnp.where(sub2 == kf, jnp.broadcast_to(wn[0, :, cols].astype(F32), (8, 256)), wr)
            wi = jnp.where(sub2 == kf, jnp.broadcast_to(wn[1, :, cols].astype(F32), (8, 256)), wi)
        yr, yi = _cmul(X[0:8], X[8:16], wr, wi)
        yield 0.1
        Y = _dot(misc[16:32, 128:256], jnp.concatenate([yr, yi, zpad], axis=0))
        br, bi = _cmul(Y[0:8], Y[8:16], twr, -twi)
        yield 0.1
        z = _dot_t(jnp.concatenate([br, bi], axis=1), _bf(CSm[...])) * 0.5
        par[1, :, 256:512] = z
        yield 0.7

    def nyq_out():
        sub = lax.broadcasted_iota(I32, (8, 128), 0)
        alt = (1 - 2 * (sub & 1)).astype(F32)
        for sf in range(8):
            for jh in range(2):
                row = jnp.broadcast_to(par[1, sf:sf + 1, _lanes(2 + jh)], (8, 128)) * alt
                Nq[sf, 128 * jh:128 * jh + 128, :] = jnp.concatenate([row] * 16, axis=0).T
                yield 1.0 / 16

    def a1(c, slot):
        for r in range(2):
            for G in range(8):
                cf = [pc[c, i] for i in range(4)]
                kv = []
                for gh in range(2):
                    j0 = 128 * r + 16 * G + 8 * gh
                    kw = [kb[c, pl.ds(8 + 4 * j0 + m, 8, stride=4), :] for m in range(4)]
                    kp = [kb[c, pl.ds(4 + 4 * j0 + m, 8, stride=4), :] for m in (2, 3)]
                    vw = [vb[c, pl.ds(4 * j0 + m, 8, stride=4), :] for m in range(4)]
                    kk = [_unpack(kp[0], 1), _unpack(kp[1], 0), _unpack(kp[1], 1)]
                    kk += [_unpack(kw[n // 2], n % 2) for n in range(8)]
                    out = []
                    for n in range(8):
                        s = (kk[n + 3] * cf[0] + kk[n + 2] * cf[1]) + (kk[n + 1] * cf[2] + kk[n] * cf[3])
                        out.append(s * _unpack(vw[n // 2], n % 2))
                    kv.append(out)
                for n in range(8):
                    Xx[slot, n, 8 * G:8 * G + 8, _lanes(r)] = _pack(kv[0][n], kv[1][n])
                yield 1.0 / 16

    def a2(c, p):
        lane = lax.broadcasted_iota(I32, (8, 128), 1)
        idx = 64 * (lane & 1) + 8 * ((lane >> 1) & 7) + (lane >> 4)
        for a in range(16):
            x = jnp.concatenate([jnp.take_along_axis(hb[c, 8 * n:8 * n + 8, _lanes(a)], idx, axis=1)
                                 for n in range(8)], axis=0)
            y = pltpu.bitcast(_bf(x).T, I32)
            for n in range(8):
                Xh[p][n, 8 * (a % 8):8 * (a % 8) + 8, _lanes(a // 8)] = y[8 * n:8 * n + 8]
            yield 1.0 / 16

    def b3(slot, p, R=64, sub=64):
        gs = Gs[p]
        for n in range(4):
            for r0 in range(0, 256, R):
                for s in range(2):
                    cols = slice(256 * s, 256 * s + 256)
                    wa, wb_ = (Xx[slot, n], Xx[slot, n + 4]) if s == 0 else (Xh[p][n], Xh[p][n + 4])
                    za = _dot(_bf(Fm[n, r0 // 2:(r0 + R) // 2, :]), _bf(wa))
                    zb = _dot(_bf(Fm[n + 4, r0 // 2:(r0 + R) // 2, :]), _bf(wb_))
                    for b in range(0, R, 8):
                        rows = slice(r0 + b, r0 + b + 8)
                        gs[n, rows, cols] = za[b:b + 8] + zb[b:b + 8]
                        gs[n + 4, rows, cols] = za[b:b + 8] - zb[b:b + 8]
                        if (b + 8) % sub == 0:
                            yield sub / 2048.0

    def b4(p, c):
        gs, yw = Gs[p], Yw[p]
        u = 1.0 / (16 * 450)
        for g in range(16):
            held = None
            for half in range(2):
                fwd, inv = (_fft4, _ifft4) if half == 0 else (_fft4o, _ifft4o)
                cost = 16 if half == 0 else 24

                def load(s):
                    return ([gs[4 * half + n, 8 * g:8 * g + 8, _lanes(s)] for n in range(4)],
                            [gs[4 * half + n, 128 + 8 * g:128 + 8 * g + 8, _lanes(s)] for n in range(4)])

                def finish(s, r, im):
                    if half == 0:
                        return r, im
                    for n in range(4):
                        yw[n, 8 * g:8 * g + 8, _lanes(s)] = _pack(held[s][0][n] + r[n], held[s][1][n] + im[n])
                        yw[n + 4, 8 * g:8 * g + 8, _lanes(s)] = _pack(held[s][0][n] - r[n], held[s][1][n] - im[n])
                x0r, x0i = fwd(*load(0))
                h1r, h1i = fwd(*load(3))
                yield 2 * cost * u
                pp = [_cmul(h1r[n], h1i[n], x0r[n], x0i[n]) for n in range(4)]
                hr, hi = load(2)
                hr[0] = hr[0] + pc[c, 4]
                h0r, h0i = fwd(hr, hi)
                yield (cost + 25) * u
                y0 = [_cmul(h0r[n], h0i[n], x0r[n], x0i[n]) for n in range(4)]
                pp = [(pp[n][0] - y0[n][1], pp[n][1] + y0[n][0]) for n in range(4)]
                yield 32 * u
                e0 = finish(0, *inv([y[0] for y in y0], [y[1] for y in y0]))
                yield (cost + 24 * half) * u
                x1r, x1i = fwd(*load(1))
                y1 = [_cmul(h0r[n], h0i[n], x1r[n], x1i[n]) for n in range(4)]
                yield (cost + 24) * u
                e1 = finish(1, *inv([y1[n][0] + pp[n][0] for n in range(4)], [y1[n][1] + pp[n][1] for n in range(4)]))
                yield (cost + 8 + 24 * half) * u
                held = (e0, e1)

    def a5(c, p, R=32, sub=32, ksplit=False, lo=0, hi=128):
        for m in range(4):
            for r0 in range(lo, hi, R):
                lhs = [Fim[2 * m + e, r0 // 2:(r0 + R) // 2, :] for e in range(2)]
                if ksplit:
                    y = [[[_dot(_bf(lhs[e][:, _lanes(kk)]), _bf(Yw[p][2 * m + e, 64 * kk:64 * kk + 64, _lanes(r)]))
                           for kk in range(2)] for e in range(2)] for r in range(2)]
                    for r in range(2):
                        for b in range(0, R, 8):
                            j0 = 128 * r + r0 + b
                            rows = pl.ds(4 * j0 + m, 8, stride=4)
                            o = [gq[c, e, rows, :] * (y[r][e][0][b:b + 8] + y[r][e][1][b:b + 8])
                                 + bb[c, 2 * m + e, j0:j0 + 8, :] for e in range(2)]
                            ob[p, rows, :] = _pack(o[0], o[1])
                            if (b + 8) % sub == 0:
                                yield sub / (8.0 * (hi - lo))
                    continue
                y = [_dot(_bf(lhs[e]), _bf(Yw[p][2 * m + e])) for e in range(2)]
                for r in range(2):
                    for b in range(0, R, 8):
                        j0 = 128 * r + r0 + b
                        rows = pl.ds(4 * j0 + m, 8, stride=4)
                        o = [gq[c, e, rows, :] * y[e][b:b + 8, _lanes(r)] + bb[c, 2 * m + e, j0:j0 + 8, :]
                             for e in range(2)]
                        ob[p, rows, :] = _pack(o[0], o[1])
                yield R / (4.0 * (hi - lo))

    nstep = [0]

    def step(*streams):
        @pl.when(pl.program_id(0) + nstep[0] <= nstep[0] if OPT["cond"] else pl.program_id(0) == 0)
        def _():
            with jax.named_scope("s%02d" % nstep[0]):
                for _ in _mix(*streams):
                    pass
        nstep[0] += 1

    def schedule():
        for name in ("gw", "sk", "d"):
            c_copy(name).start()
        c_copy("M").start()
        q_start(0)
        c_copy("G").start()
        for n in range(1, NQ):
            q_start(n)
        w_copy(0).start()
        w_copy(1).start()

        for c in range(8):
            kb[c, 0:8, :] = jnp.zeros((8, 128), I32)
        for name in ("gw", "sk", "d"):
            c_copy(name).wait()
        par[0] = jnp.broadcast_to(gwb[...].astype(F32).reshape(1, D), (8, D))
        sk = skb[...].astype(F32)
        dd = db[...].astype(F32).reshape(1, D)
        for c in range(8):
            for i in range(4):
                pc[c, i] = jnp.broadcast_to(sk[i:i + 1, _lanes(c)], (8, 128))
            pc[c, 4] = jnp.broadcast_to(dd[:, _lanes(c)], (8, 128))

        q_wait(0)
        c_copy("M").wait()
        step(p1(0, 0), make_m())
        c_copy("G").wait()
        step(expand_g())

        def phase1(it, carry):
            q_wait(2 * it + 1)
            step(p2(2 * it, 0), p1(2 * it + 1, 1))
            q_wait(2 * it + 2)
            step(p2(2 * it + 1, 1), p1(2 * it + 2, 0))
            return carry

        lax.fori_loop(0, NQ // 2 - 1, phase1, 0)
        q_wait(NQ - 1)
        step(p2(NQ - 2, 0), p1(NQ - 1, 1))
        step(p2(NQ - 1, 1), flip_m())
        t0, t1, t2, t3 = 2, 1, 3, 0
        step(p3(t0), nyq_fwd())
        step(p3(t1), p4a(t0))
        step(p3(t2), p4a(t1))
        for name in ("Gi", "CS", "misc", "wnr", "wni"):
            c_copy(name).start()
        step(p3(t3), p4a(t2))
        w_copy(0).wait()
        w_copy(1).wait()
        for which, c in ((0, 0), (1, 0), (0, 1), (1, 1), (2, 0), (2, 1), (0, 2), (1, 2)):
            a_copy(which, c).start()
        c_copy("F").start()
        a_copy(2, 2).start()
        c_copy("Fi").start()
        for c in range(3, 8):
            for which in range(3):
                a_copy(which, c).start()
        step(_chain((wprep(t0, 0), 1), (_mix(p4b(t0, 0), wprep(t1, 1)), 2)))

        def kv_wait(c):
            a_copy(0, c).wait()
            a_copy(1, c).wait()

        for name in ("Gi", "CS", "misc", "wnr", "wni"):
            c_copy(name).wait()
        step(p567(t0, 0), p4b(t1, 1), wprep(t2, 0), nyq_rest())
        kv_wait(0)
        step(p567(t1, 1), _chain((p4b(t2, 0), 4), (a1(0, 0), 3)), wprep(t3, 1), nyq_out())
        kv_wait(1)
        a_copy(2, 0).wait()
        a_copy(2, 1).wait()
        step(p567(t2, 0), _chain((p4b(t3, 1, True), 2), (a1(1, 1), 1)), _chain((a2(0, 0), 1), (a2(1, 1), 1)))
        kv_wait(2)
        c_copy("F").wait()
        step(p567(t3, 1, 64, 32, 3), b3(0, 0), a1(2, 2))
        a_copy(2, 2).wait()
        step(b3(1, 1), b4(0, 0), a2(2, 0))
        c_copy("Fi").wait()

        def steady(n, p, slot):
            kv_wait(n + 1)
            a_copy(2, n + 1).wait()
            step((_chain((b3(slot, p), 2.3), (a5(n - 2, p), 1)), 0.02),
                 _chain((b4(1 - p, n - 1), 2.6), (a1(n + 1, 1 - p), 1)), a2(n + 1, 1 - p))
            o_copy(n - 2, p).start()

        steady(2, 0, 2)

        def pair(it, carry):
            n = 3 + 2 * it

            @pl.when(it > 0)
            def _():
                o_copy(n - 4, 1).wait()
            steady(n, 1, 1)
            o_copy(n - 3, 0).wait()
            steady(n + 1, 0, 0)
            return carry

        lax.fori_loop(0, 2, pair, 0)
        o_copy(3, 1).wait()
        step((_chain((b3(1, 1), 2.3), (a5(5, 1), 1)), 0.02), b4(0, 6))
        o_copy(5, 1).start()
        o_copy(4, 0).wait()
        step(a5(6, 0), b4(1, 7))
        o_copy(6, 0).start()
        o_copy(5, 1).wait()
        step(a5(7, 1))
        o_copy(7, 1).start()
        o_copy(6, 0).wait()
        o_copy(7, 1).wait()

    pl.when(pl.program_id(0) < 1)(schedule)


@jax.jit
def pallas_gated_mix__ssm_conv_h3__spectral_gfnet__prompt_kernel(A_q, A_k, A_v, A_shift_k, A_ssm_k, A_ssm_D, B_x, B_w_r, B_w_i, gate_w):
    del B_x
    any_spec = pl.BlockSpec(memory_space=pl.ANY)
    V = pltpu.VMEM
    NQ = OPT["nq"]
    out = pl.pallas_call(
        _kernel,
        grid=(2,),
        in_specs=[any_spec] * 16,
        out_specs=any_spec,
        out_shape=jax.ShapeDtypeStruct((S, D), BF16),
        scratch_shapes=[
            V((4, 256, D), I32), V((8, 1032, 128), I32), V((8, 1024, 128), I32), V((8, 64, S), I32),
            V((2, 256, S), I32), V((2, 1024, 128), I32),
            V((4, 128, 256), I32), V((4, 64, 128), F32), V((32, 64, 128), I32), V((32, 64, 128), I32),
            V((8, 128, 128), I32), V((8, 64, 256), I32), V((128, 512), I32), V((32, 256), F32), V((11, 64, 128), I32),
            V((4, D), BF16), V((D,), BF16), V((D,), BF16), V((2, 1, S), BF16),
            V((2, 8, D), F32), V((8, 5, 8, 128), F32), V((2, 1024, 128), F32), V((8, 2, 1024, 128), F32), V((2, 1024, 128), F32),
            V((4, 1024 // NQ, 256), I32), V((4, 1024 // NQ, 256), I32), V((4, 4, 512, 128), I32),
            V((4, 4, 8, 128, 128), F32),
            V((S, 128), I32), V((S, 128), I32),
            V((4, 8, 64, 128), I32), V((4, 8, 64, 128), I32), V((3, 8, 256, 256), F32),
            V((8, 256, 128), F32), V((8, 8, 256, 128), F32),
            V((OPT["nx"], 8, 64, 256), I32), V((8, 64, 256), I32), V((8, 64, 256), I32),
            V((8, 256, 512), F32), V((8, 256, 512), F32),
            V((8, 128, 256), I32), V((8, 128, 256), I32),
            pltpu.SemaphoreType.DMA((NQ, 2)), pltpu.SemaphoreType.DMA((2,)),
            pltpu.SemaphoreType.DMA((3, 8)), pltpu.SemaphoreType.DMA((12,)), pltpu.SemaphoreType.DMA((8,)),
        ],
        compiler_params=pltpu.CompilerParams(
            vmem_limit_bytes=120 * 2 ** 20, disable_bounds_checks=True, disable_semaphore_checks=True,
            flags={"XLA_TPU_EVENLY_DISTRIBUTE_CRITICAL_NODES": True} if OPT["even"] else None),
        name="gated_mix",
    )(A_q.reshape(4, 512, D), A_k.reshape(S, D), A_v.reshape(S, D), A_ssm_k, B_w_r.T, B_w_i.T,
      A_shift_k.T, A_ssm_D, gate_w, *_CONSTS)
    return out.reshape(1, S, D)
```

```python
import numpy as np
import jax
import jax.numpy as jnp
from jax import lax
import jax.experimental.pallas as pl
import jax.experimental.pallas.tpu as pltpu

S, D = 2048, 1024
I32, F32, BF16 = jnp.int32, jnp.float32, jnp.bfloat16
RS = float(np.sqrt(0.5))
SIGN2 = int(np.array(0x80008000, np.uint32).view(np.int32))


def _w(n, N):
    return np.exp(-2j * np.pi * (np.asarray(n) % N) / N)


def _pack_rows(m):
    u = np.asarray(m, np.float32).view(np.uint32).astype(np.uint64)
    b = ((u + 0x7FFF + ((u >> 16) & 1)) >> 16).astype(np.uint32)
    return np.ascontiguousarray(b[..., 0::2, :] | (b[..., 1::2, :] << 16)).view(np.int32)


def _tile_kd(t):
    kd = np.zeros(128, np.int64)
    for lane in range(128):
        i2, r = lane // 8, lane % 8
        e = t % 2
        own = (r % 2 == 0) if e == 0 else (r % 4 in (0, 3))
        if own == (t < 2):
            i, rr = 2 * i2, r
        else:
            i, rr = 2 * i2 + 1, (r - (1 + e)) % 8
        kd[lane] = 16 * i + 8 * (rr // 4) + 2 * (rr % 4) + e
    return kd


def _make_consts():
    lo = np.stack([_tile_kd(t) % 8 == t for t in range(4)]).astype(np.int32)
    F = np.zeros((8, 256, 128))
    Fi = np.zeros((8, 128, 256))
    k1 = np.arange(128)[:, None]
    kr = np.arange(128)
    n1_of_k = 16 * (kr // 16) + 8 * (kr % 2) + (kr % 16) // 2
    for n2 in range(8):
        f = _w((8 * n1_of_k[None, :] + n2) * (4 * k1 + 1), 4096)
        F[n2, :128], F[n2, 128:] = f.real, f.imag
        fi = _w((8 * kr[None, :] + n2) * (4 * k1 + 1), 4096).T / 1024
        Fi[n2, :, 0::2], Fi[n2, :, 1::2] = fi.real, fi.imag
    jj = np.arange(256)
    cs = _w(jj[:, None] * jj[None, :], 256)
    CS = np.concatenate([cs.real, cs.imag], axis=1)
    tw = _w(np.arange(8)[:, None] * jj[None, :], 2048)
    f8 = _w(np.outer(np.arange(8), np.arange(8)), 8)
    misc = np.zeros((24, 256), np.float32)
    misc[0:8], misc[8:16] = tw.real, tw.imag
    misc[16:24, 0:8], misc[16:24, 8:16] = f8.real, f8.imag
    consts = (_pack_rows(F), _pack_rows(Fi), _pack_rows(CS), misc)
    return consts, lo


_CONSTS, _LO = _make_consts()
assert np.array_equal(_LO, np.tile(_LO[:, :8], 16))


def _unpack(x, idx):
    return pltpu.unpack_elementwise(x, index=idx, packed_dtype=BF16, unpacked_dtype=F32)


def _pack(a, b):
    return pltpu.bitcast(pltpu.pack_elementwise([a, b], packed_dtype=BF16), I32)


def _bf(x):
    return pltpu.bitcast(x, BF16)


def _dot(a, b):
    return lax.dot_general(a, b, (((1,), (0,)), ((), ())), preferred_element_type=F32)


def _dot_t(a, b):
    return lax.dot_general(a, b, (((1,), (1,)), ((), ())), preferred_element_type=F32)


def _rfft8(x):
    a0, a1, a2, a3 = x[0] + x[4], x[1] + x[5], x[2] + x[6], x[3] + x[7]
    b0, b1, nb2, b3 = x[0] - x[4], x[1] - x[5], x[6] - x[2], x[3] - x[7]
    e, o = a0 + a2, a1 + a3
    u, nv = (b1 - b3) * RS, (b1 + b3) * (-RS)
    return [(e + o, e - o), (b0 + u, nb2 + nv), (a0 - a2, a3 - a1), (b0 - u, nv - nb2)]


def _irfft8(T):
    (T0, T4), (T1r, T1i), (T2r, T2i), (T3r, T3i) = T
    a0, a1 = T0 + T4, T0 - T4
    p, q = a0 + T2r, a0 - T2r
    s, d = T1r + T3r, T1i - T3i
    u, v = T1r - T3r, T1i + T3i
    f, g = a1 - T2i, a1 + T2i
    x, y = (u - v) * RS, (u + v) * RS
    return [p + s, f + x, q - d, g - y, p - s, f - x, q + d, g + y]


def _fft4(r, i):
    ar, ai, br, bi = r[0] + r[2], i[0] + i[2], r[0] - r[2], i[0] - i[2]
    cr, ci, dr, di = r[1] + r[3], i[1] + i[3], r[1] - r[3], i[1] - i[3]
    return [ar + cr, br + di, ar - cr, br - di], [ai + ci, bi - dr, ai - ci, bi + dr]


def _ifft4(r, i):
    oi, orr = _fft4(i, r)
    return orr, oi


def _fft4o(br, bi):
    ur, ui, vr, vi = br[1] - br[3], bi[1] - bi[3], br[1] + br[3], bi[1] + bi[3]
    pr, pi = (ur + vi) * RS, (ui - vr) * RS
    qr, qi = (vr + ui) * RS, (vi - ur) * RS
    sr, si = br[0] + bi[2], bi[0] - br[2]
    tr, ti = br[0] - bi[2], bi[0] + br[2]
    return [sr + pr, tr + qi, sr - pr, tr - qi], [si + pi, ti - qr, si - pi, ti + qr]


def _ifft4o(xr, xi):
    sr, si, pr, pi = xr[0] + xr[2], xi[0] + xi[2], xr[0] - xr[2], xi[0] - xi[2]
    tr, ti, qi, qr = xr[1] + xr[3], xi[1] + xi[3], xr[1] - xr[3], xi[3] - xi[1]
    ur, ui, vr, vi = pr - qi, pi + qr, qr - pi, pr + qi
    return ([sr + tr, (ur + vr) * RS, ti - si, (vr - ur) * RS],
            [si + ti, (ui + vi) * RS, sr - tr, (vi - ui) * RS])


def _fft8(r, i):
    er, ei = _fft4([r[n] + r[n + 4] for n in range(4)], [i[n] + i[n + 4] for n in range(4)])
    orr, oi = _fft4o([r[n] - r[n + 4] for n in range(4)], [i[n] - i[n + 4] for n in range(4)])
    return [x for p in zip(er, orr) for x in p], [x for p in zip(ei, oi) for x in p]


def _ifft8(r, i):
    oi, orr = _fft8(i, r)
    return orr, oi


def _cmul(ar, ai, br, bi):
    return ar * br - ai * bi, ar * bi + ai * br


def _cis(p):
    q = (p + 256) >> 9
    x = (p - (q << 9)).astype(F32) * (np.pi / 1024)
    z = x * x
    s = x + x * z * (-1.6666654611e-1 + z * (8.3321608736e-3 + z * -1.9515295891e-4))
    c = 1.0 + z * (-0.5 + z * (4.166664568298827e-2 + z * (-1.388731625493765e-3 + z * 2.443315711809948e-5)))
    odd = (q & 1) == 1
    re, im = pltpu.bitcast(jnp.where(odd, s, c), I32), pltpu.bitcast(jnp.where(odd, c, s), I32)
    return pltpu.bitcast(re ^ (((q + 1) & 2) << 30), F32), pltpu.bitcast(im ^ ((q & 2) << 30), F32)


def _lanes(c):
    return slice(128 * c, 128 * c + 128)


def _rows8(start):
    return slice(start, start + 8)


def _span(n, size):
    return pl.ds(size * n, size)


def _mix(*streams):
    live = [list(g) if isinstance(g, tuple) else [g, 0.0] for g in streams]
    n = len(live)
    while live:
        cur = min(live, key=lambda z: z[1])
        try:
            f = next(cur[0])
        except StopIteration:
            live.remove(cur)
            continue
        cur[1] += f
        yield f / n


def _paced(stream, fraction):
    for f in stream:
        yield f * fraction


def _chain(*parts):
    total = float(sum(w for _, w in parts))
    for g, w in parts:
        for f in g:
            yield f * w / total


def _kernel(q_hbm, k_hbm, v_hbm, h_hbm, wr_hbm, wi_hbm, sk_hbm, d_hbm, gw_hbm,
            F_hbm, Fi_hbm, CS_hbm, misc_hbm,
            o_hbm,
            qb, kb, vb, hb, wb, ob, Gm, Mt, Mm, Mim, Fm, Fim, CSm, misc, Gim, skb, db, gwb, wn,
            par, pc, gate, gq, T0b, Tw, Ts, Zn, U, Wf0, Wf1, Wf2, Wf3, V0, V1, Tc, Nq, bb,
            Xx, Xh0, Xh1, Gs0, Gs1, Yw0, Yw1,
            sem_q, sem_w, sem_a, sem_c, sem_o):
    Wf, V = (Wf0, Wf1, Wf2, Wf3), (V0, V1)
    Xh, Gs, Yw = (Xh0, Xh1), (Gs0, Gs1), (Yw0, Yw1)

    def q_copy(units):
        rows = pl.ds(16 * units[0], 16 * len(units))
        return pltpu.make_async_copy(q_hbm.bitcast(I32).at[:, rows, :], qb.at[:, rows, :], sem_q.at[units[0]])

    def w_copies(a):
        return [pltpu.make_async_copy(w.at[pl.ds(0, 512), _span(a, 128)], wb.at[a, ri].bitcast(BF16), sem_w.at[a, ri])
                for ri, w in enumerate((wr_hbm, wi_hbm))]

    def a_copy(which, c):
        if which == 0:
            return pltpu.make_async_copy(k_hbm.bitcast(I32).at[:, _span(c, 128)],
                                         kb.at[c, pl.ds(8, 1024)], sem_a.at[0, c])
        if which == 1:
            return pltpu.make_async_copy(v_hbm.bitcast(I32).at[:, _span(c, 128)], vb.at[c], sem_a.at[1, c])
        return pltpu.make_async_copy(h_hbm.bitcast(I32).at[_span(c, 64), :], hb.at[c], sem_a.at[2, c])

    c_pairs = dict(F=(F_hbm, Fm), Fi=(Fi_hbm, Fim),
                   CS=(CS_hbm, CSm), misc=(misc_hbm, misc), sk=(sk_hbm, skb), d=(d_hbm, db), gw=(gw_hbm, gwb),
                   wnr=(wr_hbm.at[pl.ds(512, 1), :], wn.at[0]), wni=(wi_hbm.at[pl.ds(512, 1), :], wn.at[1]))
    c_names = list(c_pairs)

    def c_copy(name):
        src, dst = c_pairs[name]
        return pltpu.make_async_copy(src, dst, sem_c.at[c_names.index(name)])

    def o_copy(c):
        return pltpu.make_async_copy(ob.at[c], o_hbm.bitcast(I32).at[:, _span(c, 128)], sem_o.at[c])

    def own_lanes(t):
        lane = lax.broadcasted_iota(I32, (8, 128), 1)
        bits = int(sum(int(b) << n for n, b in enumerate(_LO[t][:8])))
        return ((bits >> (lane & 7)) & 1) == 1

    def make_g():
        lane = lax.broadcasted_iota(I32, (8, 128), 1)
        sub = lax.broadcasted_iota(I32, (8, 128), 0)
        for t in range(4):
            lo = own_lanes(t)
            words = [int(sum(int(k) << (8 * n) for n, k in enumerate(_tile_kd(t)[4 * h:4 * h + 4]))) for h in range(2)]
            kd = 4 * (lane & ~7) + ((jnp.where((lane & 4) == 0, words[0], words[1]) >> (8 * (lane & 3))) & 31)
            fine = [_cis(-2 * (2 * sub + e) * kd) for e in range(2)]
            Mt[8 + 2 * t], Mt[9 + 2 * t] = _cis(-32 * sub * kd)
            for n in range(8):
                if n:
                    ar = jnp.broadcast_to(Mt[8 + 2 * t, n:n + 1, :], (8, 128))
                    ai = jnp.broadcast_to(Mt[9 + 2 * t, n:n + 1, :], (8, 128))
                g = [_cmul(*f, ar, ai) if n else f for f in fine]
                gr, gi = _pack(g[0][0], g[1][0]), _pack(g[0][1], g[1][1])
                top, bot = slice(8 * n, 8 * n + 8), slice(64 + 8 * n, 72 + 8 * n)
                if t == 0:
                    Gm[t, top, 0:128], Gm[t, top, 128:256] = jnp.where(lo, gr, 0), jnp.where(lo, gi, 0)
                    Gm[t, bot, 0:128], Gm[t, bot, 128:256] = jnp.where(lo, 0, gr), jnp.where(lo, 0, gi)
                    Gim[0, top, :] = jnp.where(lo, gr, pltpu.roll(gi, 2, 1))
                    Gim[1, top, :] = jnp.where(lo, pltpu.roll(gr, 126, 1), gi)
                else:
                    Gm[t, top, 0:128], Gm[t, top, 128:256] = gr, gi
                    Gm[t, bot, 0:128] = gi ^ jnp.where(lo, SIGN2, 0)
                    Gm[t, bot, 128:256] = gr ^ jnp.where(lo, 0, SIGN2)
                    Gim[3 * t - 1, top, :] = jnp.where(lo, gr, gi)
                    Gim[3 * t, top, :] = _pack(g[0][1] - g[0][0], g[1][1] - g[1][0]) ^ jnp.where(lo, 0, SIGN2)
                    Gim[3 * t + 1, top, :] = _pack(g[0][0] + g[0][1], g[1][0] + g[1][1])
            yield 0.25

    def make_tables():
        lane = lax.broadcasted_iota(I32, (8, 128), 1)
        sub = lax.broadcasted_iota(I32, (8, 128), 0)
        for kt in range(4):
            Mt[2 * kt], Mt[2 * kt + 1] = _cis(sub * (kt + 4 * (lane >> 1)))
        yield 1.0

    def make_m():
        lane = lax.broadcasted_iota(I32, (8, 128), 1)
        sub = lax.broadcasted_iota(I32, (8, 128), 0)
        sm, km4 = 4 * (sub & 3) + (sub >> 2), 4 * (lane >> 1)
        base, step16, step2 = [_cis(8 * sm * km4 + 512 * (lane & 1))], _cis(128 * km4), _cis(16 * km4)
        for r in range(7):
            base.append(_cmul(*base[r], *step16) if r < 3 else _cmul(*base[r - 3], *step2))
        turn0 = _cis(8 * sm)
        turn = [_cmul(*turn0, float(w.real), float(w.imag)) if r else turn0
                for r, w in enumerate(_w(-(16 * (np.arange(8) % 4) + 2 * (np.arange(8) // 4)), 256))]
        for kt in range(4):
            if kt:
                base = [_cmul(*b, *w) for b, w in zip(base, turn)]
            for sf in range(8):
                n = 8 * kt + sf
                br = jnp.broadcast_to(Mt[2 * kt, sf:sf + 1, :], (8, 128))
                bi = jnp.broadcast_to(Mt[2 * kt + 1, sf:sf + 1, :], (8, 128))
                rows, ordered = [], []
                for b in range(4):
                    er, ei = _cmul(*base[b], br, bi) if sf else base[b]
                    orr, oi = _cmul(*base[4 + b], br, bi) if sf else base[4 + b]
                    rows += [_pack(er, orr), _pack(ei, oi)]
                    lo, hi = _pack(er, ei), _pack(orr, oi)
                    for half in range(2):
                        idx = ((sub & 1) << 2) + (sub >> 2) + 2 * half
                        ordered.append(jnp.where((sub & 2) == 0, jnp.take_along_axis(lo, idx, axis=0),
                                                 jnp.take_along_axis(hi, idx, axis=0)))
                Mm[n] = pltpu.bitcast(_bf(jnp.concatenate(ordered, axis=0)).T, I32)
                for r in range(8):
                    Mim[n, 8 * r:8 * r + 8, :] = rows[r]
                yield 1.0 / 32

    def flip_g():
        for n in range(11):
            Gim[n] = pltpu.bitcast(_bf(Gim[n]).T, I32)
            yield 1.0 / 11

    def p1(units, lean=()):
        for i in [2 * n + il for n in units for il in range(2)]:
            for st in range(4):
                prow = _rows8(256 * st + 8 * i)
                xw = [qb[st, _rows8(8 * i), _lanes(c)] for c in range(8)]
                T = []
                for e in range(2):
                    x = [_unpack(w, e) for w in xw]
                    pr = [x[c] * par[0, :, _lanes(c)] for c in range(8)]
                    acc = ((pr[0] + pr[1]) + (pr[2] + pr[3])) + ((pr[4] + pr[5]) + (pr[6] + pr[7]))
                    th = 0.5 * jnp.tanh(0.5 * jnp.broadcast_to(jnp.sum(acc, axis=1, keepdims=True), (8, 128)))
                    g = 0.5 + th
                    gate[e, prow, :] = (0.5 - th) * 2.0 ** -20
                    for c in range(8):
                        gq[c, e, prow, :] = x[c] * g
                    T.append(_rfft8(x))
                    T0b[e, prow, :] = T[e][0][0]
                    yield 1.0 / (16 * len(units))
                r0 = 32 * (i % 2) + 8 * st
                for t in range(4):
                    for h in range(2):
                        Tw[i // 2, t, r0:r0 + 8, _lanes(h)] = _pack(T[0][t][h], T[1][t][h])
                for t in lean:
                    Ts[i // 2, t - 1, r0:r0 + 8, :] = _pack(T[0][t][0] + T[0][t][1], T[1][t][0] + T[1][t][1])

    def p2(units, lean=(), order=range(4), together=False):
        for t in order:
            lo = own_lanes(t)
            for part in [units] if together else [(n,) for n in units]:
                x = jnp.concatenate([Tw[n, t] for n in part], axis=0)
                if t not in lean:
                    z = _dot(_bf(x), _bf(Gm[t]))
                elif t == 0:
                    za, zb = [_dot(_bf(x[:, _lanes(h)]), _bf(Gim[h])) for h in range(2)]
                else:
                    zs = _dot(_bf(jnp.concatenate([Ts[n, t - 1] for n in part], axis=0)), _bf(Gim[3 * t - 1]))
                    za = _dot(_bf(x[:, 128:256]), _bf(Gim[3 * t + 1]))
                    zb = _dot(_bf(x[:, 0:128]), _bf(Gim[3 * t]))
                for ii in range(2 * len(part)):
                    for u in range(2):
                        rows = [_rows8(64 * ii + 16 * st + 8 * u) for st in range(4)]
                        if t not in lean:
                            r, im = [z[s, 0:128] for s in rows], [z[s, 128:256] for s in rows]
                        elif t == 0:
                            r = [jnp.where(lo, za[s], pltpu.roll(zb[s], 2, 1)) for s in rows]
                            im = [jnp.where(lo, pltpu.roll(za[s], 126, 1), zb[s]) for s in rows]
                        else:
                            o1, o2 = [zs[s] - za[s] for s in rows], [zs[s] + zb[s] for s in rows]
                            r = [jnp.where(lo, a, b) for a, b in zip(o1, o2)]
                            im = [jnp.where(lo, b, a) for a, b in zip(o1, o2)]
                        r, im = _fft4(r, im)
                        for kt in range(4):
                            Zn[t, kt, _rows8(32 * part[0] + 16 * ii + 8 * u), :] = _pack(r[kt], im[kt])
                yield 0.25 * len(part) / len(units)

    def p3(t, R=64, every=1):
        for kt in range(4):
            for sf in range(8):
                x = _bf(Zn[t, kt, pl.ds(sf, 64, stride=8), :])
                for r0 in range(0, 128, R):
                    U[t, kt, sf, r0:r0 + R, :] = _dot(_bf(Mm[8 * kt + sf, r0 // 2:(r0 + R) // 2, :]), x)
                if (sf + 1) % every == 0:
                    yield every / 32

    def p4a(t):
        for kt in range(4):
            for g in range(8):
                re, im = pl.ds(16 * g, 8, stride=2), pl.ds(16 * g + 1, 8, stride=2)
                r, i = _fft8([U[t, kt, sf, re, :] for sf in range(8)], [U[t, kt, sf, im, :] for sf in range(8)])
                for kf in range(8):
                    U[t, kt, kf, 16 * g:16 * g + 8, :] = r[kf]
                    U[t, kt, kf, 16 * g + 8:16 * g + 16, :] = i[kf]
                yield 1.0 / 32

    def wprep(work):
        sub = lax.broadcasted_iota(I32, (8, 128), 0)
        for a, e in work:
            own = ((sub & 1) == 0) if e == 0 else (((sub + 1) & 2) == 0)
            rows = ([], [])
            for i2 in range(16):
                words = []
                for r0 in (16 * i2, 16 * i2 + 8):
                    x = [wb[a, ri, r0:r0 + 8, :] for ri in range(2)]
                    if e == 0 and r0 == 0:
                        half = jnp.where(sub == 0, 0.5, 1.0)
                        words.append(_pack(_unpack(x[0], e) * half, _unpack(x[1], e) * half))
                    elif e == 0:
                        words.append(pltpu.bitcast(pltpu.pack_elementwise(x, packed_dtype=jnp.int16), I32))
                    else:
                        words.append(_pack(_unpack(x[0], e), _unpack(x[1], e)))
                A, B = words[0], pltpu.roll(words[1], 1 + e, 0)
                rows[0].append(jnp.where(own, A, B))
                rows[1].append(jnp.where(own, B, A))
            for h in range(2):
                Wf[e + 2 * h][128 * a:128 * a + 128, :] = jnp.concatenate(rows[h], axis=0).T
            yield 1.0 / len(work)

    def p4b(t, p, full=True, groups=range(8)):
        w, v = Wf[t], V[p]
        u = 1.0 / ((12 if full else 8) * len(groups))
        for g in groups:
            for kt in range(4):
                if full:
                    re, ie = pl.ds(16 * g, 8, stride=2), pl.ds(16 * g + 1, 8, stride=2)
                else:
                    re, ie = slice(16 * g, 16 * g + 8), slice(16 * g + 8, 16 * g + 16)
                r = [U[t, kt, n, re, :] for n in range(8)]
                im = [U[t, kt, n, ie, :] for n in range(8)]
                if full:
                    r, im = _fft8(r, im)
                    yield u
                for kf in range(8):
                    ww = w[pl.ds(256 * kf + 32 * g + kt, 8, stride=4), :]
                    r[kf], im[kf] = _cmul(r[kf], im[kf], _unpack(ww, 0), _unpack(ww, 1))
                yield u
                r, im = _ifft8(r, im)
                for sf in range(8):
                    v[kt, sf, 8 * g:8 * g + 8, :] = _pack(r[sf], im[sf])
                yield u

    def r567(t, p, m6, look):
        lo = own_lanes(t)
        cost6 = 2.0 if t == 0 else 3.0
        total = 8 * (128 + 64 * cost6)

        def first(sf, h):
            o = {kt: _dot(_bf(Mim[8 * kt + sf, 32 * h:32 * h + 32, :]), _bf(V[p][kt, sf]))
                 for kt in (range(4) if t else (0, 2, 1, 3))}
            o = [o[kt] for kt in range(4)]
            la, lb, ls, dest = [], [], [], []
            for b in range(2):
                r, im = zip(*[_ifft4([x[32 * b + 8 * u:32 * b + 8 * u + 8] for x in o],
                                     [x[32 * b + 16 + 8 * u:32 * b + 24 + 8 * u] for x in o]) for u in range(2)])
                for st in range(4):
                    wr, wi = _pack(r[0][st], r[1][st]), _pack(im[0][st], im[1][st])
                    if t == 0:
                        la.append(jnp.where(lo, wr, pltpu.roll(wi, 2, 1)))
                        lb.append(jnp.where(lo, pltpu.roll(wr, 126, 1), wi))
                    else:
                        la.append(jnp.where(lo, wr, wi))
                        lb.append(jnp.where(lo, wi, wr))
                        ls.append(_pack(r[0][st] + im[0][st], r[1][st] + im[1][st]))
                    dest += [64 * st + 32 * h + 16 * b, 64 * st + 32 * h + 16 * b + 8]
            return sf, la, lb, ls, dest

        def second(sf, la, lb, ls, dest):
            for part in range(128 // m6):
                sel = slice(part * m6 // 16, (part + 1) * m6 // 16)
                xa, xb = _bf(jnp.concatenate(la[sel], axis=0)), _bf(jnp.concatenate(lb[sel], axis=0))
                if t == 0:
                    yi, yr = _dot(xb, _bf(Gim[1])), _dot(xa, _bf(Gim[0]))
                else:
                    yq = _dot(xb, _bf(Gim[3 * t]))
                    yp = _dot(_bf(jnp.concatenate(ls[sel], axis=0)), _bf(Gim[3 * t - 1]))
                    ys = _dot(xa, _bf(Gim[3 * t + 1]))
                for n, j0 in enumerate(dest[part * m6 // 8:(part + 1) * m6 // 8]):
                    r8 = slice(8 * n, 8 * n + 8)
                    tr, ti = (yr[r8], yi[r8]) if t == 0 else (yp[r8] + yq[r8], yp[r8] - ys[r8])
                    rows = slice(j0, j0 + 8)
                    if t > 0:
                        Tc[t - 1, sf, rows, 0:128] = tr
                        Tc[t - 1, sf, rows, 128:256] = ti
                    else:
                        T = [(Tc[tt, sf, rows, 0:128], Tc[tt, sf, rows, 128:256]) for tt in range(3)]
                        b_ = _irfft8([(tr + Nq[sf, rows, :], ti)] + T)
                        omg = gate[sf % 2, pl.ds(4 * j0 + sf // 2, 8, stride=4), :]
                        for c in range(8):
                            bb[c, sf, rows, :] = b_[c] * omg
                yield (m6 / 2 + m6 * cost6 / 4) / total

        pend = []
        for sf in range(8):
            for h in range(2):
                pend.append(first(sf, h))
                if len(pend) > look:
                    yield from second(*pend.pop(0))
        while pend:
            yield from second(*pend.pop(0))

    def nyq_fwd():
        sub = lax.broadcasted_iota(I32, (8, 128), 0)
        alt = (1 - 2 * (sub & 1)).astype(F32)
        for jh in range(2):
            acc = jnp.zeros((8, 128), F32)
            for sf in range(8):
                tile = T0b[sf % 2, pl.ds(512 * jh + sf // 2, 128, stride=4), :].T
                s = tile[0:8]
                for n in range(1, 16):
                    s = s + tile[8 * n:8 * n + 8]
                s = jnp.sum(s * alt, axis=0, keepdims=True)
                acc = jnp.where(sub == sf, jnp.broadcast_to(s, (8, 128)), acc)
                yield 1.0 / 16
            par[1, :, _lanes(jh)] = acc

    def nyq_dft():
        par[1, :, 512:1024] = _dot(par[1, :, 0:256], _bf(CSm[...]))
        yield 1.0

    def nyq_filter():
        tab = misc[16:24, 0:128]
        w8 = [[jnp.take_along_axis(tab, jnp.full((8, 128), 8 * ri + r, I32), axis=1) for ri in range(2)]
              for r in range(8)]

        def dft8(xr, xi, sign):
            accr = acci = None
            for r in range(8):
                pr, pi = _cmul(jnp.broadcast_to(xr[r:r + 1], (8, 128)), jnp.broadcast_to(xi[r:r + 1], (8, 128)),
                               w8[r][0], w8[r][1] * sign)
                accr, acci = (pr, pi) if r == 0 else (accr + pr, acci + pi)
            return accr, acci

        sub = lax.broadcasted_iota(I32, (8, 128), 0)
        out = []
        for c in range(2):
            twr, twi = misc[0:8, _lanes(c)], misc[8:16, _lanes(c)]
            wr = wi = jnp.zeros((8, 128), F32)
            for kf in range(8):
                cols = _lanes(2 * kf + c)
                wr = jnp.where(sub == kf, jnp.broadcast_to(wn[0, :, cols].astype(F32), (8, 128)), wr)
                wi = jnp.where(sub == kf, jnp.broadcast_to(wn[1, :, cols].astype(F32), (8, 128)), wi)
            x = dft8(*_cmul(par[1, :, _lanes(4 + c)], par[1, :, _lanes(6 + c)], twr, twi), 1.0)
            y = dft8(*_cmul(*x, wr, wi), -1.0)
            out.append(_cmul(*y, twr, -twi))
            yield 0.3
        lhs = jnp.concatenate([out[0][0], out[1][0], out[0][1], out[1][1]], axis=1)
        par[1, :, 256:512] = _dot_t(lhs, _bf(CSm[...])) * 0.5
        yield 0.4

    def nyq_out():
        sub = lax.broadcasted_iota(I32, (8, 128), 0)
        alt = (1 - 2 * (sub & 1)).astype(F32)
        for sf in range(8):
            for jh in range(2):
                row = jnp.broadcast_to(par[1, sf:sf + 1, _lanes(2 + jh)], (8, 128)) * alt
                Nq[sf, 128 * jh:128 * jh + 128, :] = jnp.concatenate([row] * 16, axis=0).T
                yield 1.0 / 16

    def a1(c, slot):
        for part in range(16):
            G, r = divmod(part, 2)
            cf = [pc[c, i] for i in range(4)]
            kv = []
            for gh in range(2):
                j0 = 128 * r + 16 * G + 8 * gh
                kw = [kb[c, pl.ds(8 + 4 * j0 + m, 8, stride=4), :] for m in range(4)]
                kp = [kb[c, pl.ds(4 + 4 * j0 + m, 8, stride=4), :] for m in (2, 3)]
                vw = [vb[c, pl.ds(4 * j0 + m, 8, stride=4), :] for m in range(4)]
                kk = [_unpack(kp[0], 1), _unpack(kp[1], 0), _unpack(kp[1], 1)]
                kk += [_unpack(kw[n // 2], n % 2) for n in range(8)]
                out = []
                for n in range(8):
                    s = (kk[n + 3] * cf[0] + kk[n + 2] * cf[1]) + (kk[n + 1] * cf[2] + kk[n] * cf[3])
                    out.append(s * _unpack(vw[n // 2], n % 2))
                kv.append(out)
                if gh == 0:
                    yield 1.0 / 32
            for n in range(8):
                Xx[slot, n, 8 * G:8 * G + 8, _lanes(r)] = _pack(kv[0][n], kv[1][n])
            yield 1.0 / 32

    def a2(c, p):
        lane = lax.broadcasted_iota(I32, (8, 128), 1)
        idx = 64 * (lane & 1) + 8 * ((lane >> 1) & 7) + (lane >> 4)
        for a in range(16):
            x = jnp.concatenate([jnp.take_along_axis(hb[c, 8 * n:8 * n + 8, _lanes(a)], idx, axis=1)
                                 for n in range(8)], axis=0)
            y = pltpu.bitcast(_bf(x).T, I32)
            for n in range(8):
                Xh[p][n, 8 * (a % 8):8 * (a % 8) + 8, _lanes(a // 8)] = y[8 * n:8 * n + 8]
            yield 1.0 / 16

    def b3(slot, p, order="rns"):
        gs = Gs[p]
        pieces = [dict(n=n, r=r, s=s) for n in range(4) for r in range(4) for s in range(2)]
        for piece in sorted(pieces, key=lambda z: [z[k] for k in order]):
            n, r, s = piece["n"], piece["r"], piece["s"]
            cols = slice(256 * s, 256 * s + 256)
            wa, wb_ = (Xx[slot, n], Xx[slot, n + 4]) if s == 0 else (Xh[p][n], Xh[p][n + 4])
            zb = _dot(_bf(Fm[n + 4, 32 * r:32 * r + 32, :]), _bf(wb_))
            za = _dot(_bf(Fm[n, 32 * r:32 * r + 32, :]), _bf(wa))
            for b in range(0, 64, 8):
                rows = _rows8(64 * r + b)
                gs[n + 4, rows, cols] = za[b:b + 8] - zb[b:b + 8]
                gs[n, rows, cols] = za[b:b + 8] + zb[b:b + 8]
            yield 1.0 / 32

    def b4(p, c, groups=range(16)):
        gs, yw = Gs[p], Yw[p]
        u = 1.0 / (len(groups) * 450)
        for g in groups:
            held = None
            for half in range(2):
                fwd, inv = (_fft4, _ifft4) if half == 0 else (_fft4o, _ifft4o)
                cost = 16 if half == 0 else 24

                def load(s):
                    return ([gs[4 * half + n, 8 * g:8 * g + 8, _lanes(s)] for n in range(4)],
                            [gs[4 * half + n, 128 + 8 * g:128 + 8 * g + 8, _lanes(s)] for n in range(4)])

                def finish(s, r, im):
                    if half == 0:
                        return r, im
                    (er, ei), (orr, oi) = held[s], (r, im)
                    for n in range(4):
                        yw[n + 4, 8 * g:8 * g + 8, _lanes(s)] = _pack(er[n] - orr[n], ei[n] - oi[n])
                        yw[n, 8 * g:8 * g + 8, _lanes(s)] = _pack(er[n] + orr[n], ei[n] + oi[n])
                x0r, x0i = fwd(*load(0))
                h1r, h1i = fwd(*load(3))
                yield 2 * cost * u
                pp = [_cmul(h1r[n], h1i[n], x0r[n], x0i[n]) for n in range(4)]
                hr, hi = load(2)
                hr[0] = hr[0] + pc[c, 4]
                h0r, h0i = fwd(hr, hi)
                yield (cost + 25) * u
                y0 = [_cmul(h0r[n], h0i[n], x0r[n], x0i[n]) for n in range(4)]
                pp = [(pp[n][0] - y0[n][1], pp[n][1] + y0[n][0]) for n in range(4)]
                yield 32 * u
                e0 = finish(0, *inv([y[0] for y in y0], [y[1] for y in y0]))
                yield (cost + 24 * half) * u
                x1r, x1i = fwd(*load(1))
                y1 = [_cmul(h0r[n], h0i[n], x1r[n], x1i[n]) for n in range(4)]
                yield (cost + 24) * u
                e1 = finish(1, *inv([y1[n][0] + pp[n][0] for n in range(4)], [y1[n][1] + pp[n][1] for n in range(4)]))
                yield (cost + 8 + 24 * half) * u
                held = (e0, e1)

    def c5(c, p, R):
        for m in range(4):
            for r in range(2):
                for r0 in range(0, 128, R):
                    y = [_dot(_bf(Fim[2 * m + e, r0 // 2:(r0 + R) // 2, :]), _bf(Yw[p][2 * m + e, :, _lanes(r)]))
                         for e in range(2)]
                    for b in range(0, R, 8):
                        j0 = 128 * r + r0 + b
                        rows = pl.ds(4 * j0 + m, 8, stride=4)
                        o = [gq[c, e, rows, :] * y[e][b:b + 8] + bb[c, 2 * m + e, j0:j0 + 8, :] for e in range(2)]
                        ob[c, rows, :] = _pack(o[0], o[1])
                    yield R / 1024.0

    def c5_head():
        for n in range(8):
            Gs[0][n, 0:128, 0:256] = _dot(_bf(Fim[n, :, 0:128]), _bf(Yw1[n, 0:64, :]))
            yield 1.0 / 8

    def c5_tail(c, r, lo, hi):
        half = max((hi - lo) // 2, 32)
        for m in range(4):
            y = [_dot(_bf(Fim[2 * m + e, (lo + half * h) // 2:(lo + half * (h + 1)) // 2, 128:256]),
                      _bf(Yw1[2 * m + e, 64:128, _lanes(r)])) for h in range((hi - lo) // half) for e in range(2)]
            for b in range(0, hi - lo, 8):
                j0 = 128 * r + lo + b
                rows = pl.ds(4 * j0 + m, 8, stride=4)
                o = [gq[c, e, rows, :] * (y[2 * (b // half) + e][b % half:b % half + 8]
                                          + Gs[0][2 * m + e, lo + b:lo + b + 8, _lanes(r)])
                     + bb[c, 2 * m + e, j0:j0 + 8, :] for e in range(2)]
                ob[c, rows, :] = _pack(o[0], o[1])
            yield 1.0 / 4

    nstep = [0]

    def step(*streams):
        @pl.when(pl.program_id(0) + nstep[0] <= nstep[0])
        def _():
            for _ in _mix(*streams):
                pass
        nstep[0] += 1

    def fetch(*copies):
        for c in copies:
            c.start()
            yield 1.0 / len(copies)

    def wait(*copies):
        for c in copies:
            c.wait()

    def block_copies(c):
        return [a_copy(which, c) for which in range(3)]

    def coefficients():
        for c in range(8):
            kb[c, 0:8, :] = jnp.zeros((8, 128), I32)
        sk = skb[...].astype(F32)
        dd = db[...].astype(F32).reshape(1, D)
        for c in range(8):
            for i in range(4):
                pc[c, i] = jnp.broadcast_to(sk[i:i + 1, _lanes(c)], (8, 128))
            pc[c, 4] = jnp.broadcast_to(dd[:, _lanes(c)], (8, 128))
            yield 1.0 / 8

    @pl.when(pl.program_id(0) < 1)
    def _():
        units = [(0,), (1,)] + [(n, n + 1) for n in range(2, 16, 2)]
        blocks = list(range(0, 16, 2)) + list(range(1, 16, 2))
        step(fetch(c_copy("gw"), c_copy("sk"), c_copy("d"), q_copy(units[0])))
        step(fetch(*[q_copy(n) for n in units[1:]]))
        step(make_g(), make_tables())
        step(make_m(), fetch(*[c for a in blocks for c in w_copies(a)]))
        wait(c_copy("gw"))
        par[0] = jnp.broadcast_to(gwb[...].astype(F32).reshape(1, D), (8, D))
        wait(q_copy(units[0]))
        step(p1(units[0], (1, 3)))
        wait(q_copy(units[1]))
        step(p2(units[0], (1, 3)), p1(units[1]))
        wait(q_copy(units[2]))
        step(p2(units[1]), p1(units[2], (1, 3)))
        for n in range(2, 8):
            wait(q_copy(units[n + 1]))
            step(p2(units[n], (1, 3)), p1(units[n + 1], (1, 3) if n < 7 else (1, 2, 3)))
        wait(c_copy("sk"), c_copy("d"))
        step(p2(units[8], range(4), (1, 0, 2, 3), True), coefficients())

        def w_arrived(lo, hi):
            wait(*[c for a in blocks[lo:hi] for c in w_copies(a)])
            return [(a, 1) for a in blocks[lo:hi]]

        def even_rows(lo, hi):
            return [(a, 0) for a in blocks[lo:hi]]

        step(_chain((p3(1), 1), (p3(3), 1)), _paced(_chain((nyq_fwd(), 3), (flip_g(), 1)), 0.746),
             _paced(wprep(w_arrived(0, 5) + even_rows(0, 5)), 0.761))
        step((p3(2), 0.007), _paced(wprep(w_arrived(5, 8) + even_rows(5, 8)), 0.632), (p4a(1), 0.051))
        step(fetch(c_copy("CS"), a_copy(0, 0), a_copy(1, 0), c_copy("misc"), c_copy("wnr"), c_copy("wni"), a_copy(2, 0),
                   *block_copies(1), a_copy(0, 2), a_copy(1, 2), c_copy("F"), a_copy(2, 2), c_copy("Fi")))
        step((p3(0, 128, 2), 0.008), _chain((p4a(2), 1), (p4b(1, 0, False, range(4)), 1.101)),
             _paced(wprep(w_arrived(8, 12)), 0.719))
        step(fetch(*[c for n in range(3, 8) for c in block_copies(n)]))
        step(_chain((wprep(w_arrived(12, 16)), 1), (p4b(1, 0, False, range(4, 8)), 2)))

        step((r567(1, 0, 32, 1), 0.044), (_paced(p4b(3, 1), 0.995), 0.044), _paced(wprep(even_rows(8, 16)), 0.415))
        wait(a_copy(0, 0), a_copy(1, 0), c_copy("CS"))
        step((r567(3, 1, 32, 1), 0.073), _chain((a1(0, 0), 16), (p4b(2, 0, False), 21.333), (nyq_dft(), 1.098)))
        wait(a_copy(2, 0), c_copy("misc"), c_copy("wnr"), c_copy("wni"))
        step(_paced(p4b(0, 1), 1.003), _chain((nyq_filter(), 0.188), (a2(0, 0), 1), (nyq_out(), 0.959)),
             (r567(2, 0, 32, 1), 0.005))
        step(r567(0, 1, 128, 3))

        wait(*block_copies(1), a_copy(0, 2), a_copy(1, 2), c_copy("F"))
        step((b3(0, 0, "nrs"), 0.003), _paced(_chain((a1(1, 1), 1), (a1(2, 2), 1)), 0.99), _paced(a2(1, 1), 0.753))
        wait(a_copy(2, 2))
        step((b3(1, 1, "snr"), 0.041), _paced(a2(2, 0), 0.75), (b4(0, 0), 0.003))
        wait(c_copy("Fi"))
        for n in range(2, 7):
            wait(*block_copies(n + 1))
            if n == 6:
                for c in range(4):
                    o_copy(c).start()
            p = n % 2
            step((_paced(_chain((a1(n + 1, 1 - p), 1), (b4(1 - p, n - 1), 2.881)), 0.982), 0.022),
                 _paced(a2(n + 1, 1 - p), 0.576),
                 (_mix((b3(2 if n == 2 else p, p), 0.001), (_paced(c5(n - 2, p, 32), 1.025), 0.07)), 0.018))
        o_copy(4).start()
        step((_paced(b4(0, 6), 0.978), 0.035), (_mix(b3(1, 1), c5(5, 1, 32)), 0.033))
        o_copy(5).start()
        step((b4(1, 7, range(0, 8)), 0.002), (c5(6, 0, 64), 0.083))
        o_copy(6).start()
        step(b4(1, 7, range(8, 16)), _paced(c5_head(), 1.011))
        last = []
        for n, parts in enumerate(([(0, 0, 96)], [(0, 96, 128), (1, 0, 64)], [(1, 64, 128)])):
            step(_chain(*[(c5_tail(7, r, lo, hi), hi - lo) for r, lo, hi in parts]))
            rows = pl.ds(512 * parts[0][0] + 4 * parts[0][1], 4 * sum(hi - lo for _, lo, hi in parts))
            last.append(pltpu.make_async_copy(ob.at[7, rows], o_hbm.bitcast(I32).at[rows, _span(7, 128)],
                                              sem_o.at[7 + n]))
            last[-1].start()
        wait(*[o_copy(c) for c in range(7)], *last)


@jax.jit
def pallas_gated_mix__ssm_conv_h3__spectral_gfnet__prompt_kernel(A_q, A_k, A_v, A_shift_k, A_ssm_k, A_ssm_D, B_x, B_w_r, B_w_i, gate_w):
    del B_x
    any_spec = pl.BlockSpec(memory_space=pl.ANY)
    V = pltpu.VMEM
    out = pl.pallas_call(
        _kernel,
        grid=(2,),
        in_specs=[any_spec] * 13,
        out_specs=any_spec,
        out_shape=jax.ShapeDtypeStruct((S, D), BF16),
        scratch_shapes=[
            V((4, 256, D), I32), V((8, 1056, 128), I32), V((8, 1024, 128), I32), V((8, 64, S), I32),
            V((16, 2, 256, 128), I32), V((8, 1024, 128), I32),
            V((4, 128, 256), I32), V((16, 8, 128), F32), V((32, 64, 128), I32), V((32, 64, 128), I32),
            V((8, 128, 128), I32), V((8, 64, 256), I32), V((128, 512), I32), V((24, 256), F32), V((11, 64, 128), I32),
            V((4, D), BF16), V((D,), BF16), V((D,), BF16), V((2, 1, S), BF16),
            V((2, 8, D), F32), V((8, 8, 8, 128), F32), V((2, 1024, 128), F32), V((8, 2, 1024, 128), F32), V((2, 1024, 128), F32),
            V((16, 4, 64, 256), I32), V((16, 3, 64, 128), I32), V((4, 4, 512, 128), I32),
            V((4, 4, 8, 128, 128), F32),
            V((S, 128), I32), V((S, 128), I32), V((S, 128), I32), V((S, 128), I32),
            V((4, 8, 64, 128), I32), V((4, 8, 64, 128), I32), V((3, 8, 256, 256), F32),
            V((8, 256, 128), F32), V((8, 8, 256, 128), F32),
            V((3, 8, 64, 256), I32), V((8, 64, 256), I32), V((8, 64, 256), I32),
            V((8, 256, 512), F32), V((8, 256, 512), F32),
            V((8, 128, 256), I32), V((8, 128, 256), I32),
            pltpu.SemaphoreType.DMA((16,)), pltpu.SemaphoreType.DMA((16, 2)),
            pltpu.SemaphoreType.DMA((3, 8)), pltpu.SemaphoreType.DMA((9,)), pltpu.SemaphoreType.DMA((10,)),
        ],
        compiler_params=pltpu.CompilerParams(
            vmem_limit_bytes=120 * 2 ** 20, disable_bounds_checks=True, disable_semaphore_checks=True,
            flags={"XLA_TPU_EVENLY_DISTRIBUTE_CRITICAL_NODES": True}),
        name="gated_mix",
    )(A_q.reshape(4, 512, D), A_k.reshape(S, D), A_v.reshape(S, D), A_ssm_k, B_w_r.T, B_w_i.T,
      A_shift_k.T, A_ssm_D, gate_w, *_CONSTS)
    return out.reshape(1, S, D)
```
